```python
import jax
import jax.numpy as jnp

def _softmax(x, axis=-1):
    return jax.nn.softmax(x, axis=axis)

def _gelu(x):
    return jax.nn.gelu(x, approximate=True)

def _silu(x):
    return jax.nn.silu(x)

def _sigmoid(x):
    return jax.nn.sigmoid(x)

def _layernorm(x, axis=-1, eps=1e-05):
    m = jnp.mean(x, axis=axis, keepdims=True)
    v = jnp.var(x, axis=axis, keepdims=True)
    return (x - m) / jnp.sqrt(v + eps)

def _scatter_add(tgt, idx, src, axis=0):
    return tgt.at[idx].add(src)

def _segment_sum(src, seg, n):
    return jax.ops.segment_sum(src, seg, n)

class _Rng:

    def __init__(self, key):
        self._k = key

    def _next(self):
        self._k, sub = jax.random.split(self._k)
        return sub

    def normal(self, shape):
        return jax.random.normal(self._next(), shape, dtype=jnp.bfloat16)

    def randint(self, lo, hi, shape):
        return jax.random.randint(self._next(), shape, lo, hi, dtype=jnp.int32)

    def uniform(self, shape, lo=0.0, hi=1.0):
        return jax.random.uniform(self._next(), shape, jnp.bfloat16, lo, hi)

    def permutation(self, n):
        return jax.random.permutation(self._next(), n)
kernel_name = 'interleave_layers__memory_aug_infini_attn__mixer_s_mlp__prompt'

def setup_inputs():
    _rng = _Rng(jax.random.key(int.from_bytes(__import__("os").urandom(4), "little")))
    _w = lambda a: (lambda t: t.astype(jnp.bfloat16) if jnp.issubdtype(t.dtype, jnp.floating) else t)(jnp.asarray(a))

    def _A_setup():
        B, S, D, H = (1, 2048, 1024, 32)
        N = 4
        L = max(1, S // N)
        sc = D ** (-0.5)
        return {'x': _w((lambda *s: _rng.normal(s) * 0.05)(B, N * L, D)), 'wq': _w((lambda *s: _rng.normal(s) * 0.05)(D, D) * sc), 'wk': _w((lambda *s: _rng.normal(s) * 0.05)(D, D) * sc), 'wv': _w((lambda *s: _rng.normal(s) * 0.05)(D, D) * sc), 'wo': _w((lambda *s: _rng.normal(s) * 0.05)(D, D) * sc), 'beta': _w((lambda *s: _rng.normal(s) * 0.05)(H))}
    _A_in = _A_setup()

    def _B_setup():
        B, S, D, F = (1, 2048, 1024, 3584)
        return {'x': _w((lambda *s: _rng.normal(s) * 0.05)(B, S, D)), 'w1': _w((lambda *s: _rng.normal(s) * 0.05)(D, D) * D ** (-0.5)), 'w2': _w((lambda *s: _rng.normal(s) * 0.05)(D, D) * D ** (-0.5)), 'w3': _w((lambda *s: _rng.normal(s) * 0.05)(D, F) * D ** (-0.5)), 'w4': _w((lambda *s: _rng.normal(s) * 0.05)(F, D) * F ** (-0.5))}
    _B_in = _B_setup()
    return {'A_x': _A_in['x'], 'A_wq': _A_in['wq'], 'A_wk': _A_in['wk'], 'A_wv': _A_in['wv'], 'A_wo': _A_in['wo'], 'A_beta': _A_in['beta'], 'B_x': _B_in['x'], 'B_w1': _B_in['w1'], 'B_w2': _B_in['w2'], 'B_w3': _B_in['w3'], 'B_w4': _B_in['w4']}

def reference(A_x, A_wq, A_wk, A_wv, A_wo, A_beta, B_x, B_w1, B_w2, B_w3, B_w4):

    def _A_ref(x, wq, wk, wv, wo, beta):
        B, S, D = x.shape
        H = 32
        Dh = D // H
        N = 4
        L = S // N
        q = (lambda x, *d: x.transpose(*d))((x @ wq).reshape(B, S, H, Dh), 0, 2, 1, 3).reshape(B, H, N, L, Dh)
        k = (lambda x, *d: x.transpose(*d))((x @ wk).reshape(B, S, H, Dh), 0, 2, 1, 3).reshape(B, H, N, L, Dh)
        v = (lambda x, *d: x.transpose(*d))((x @ wv).reshape(B, S, H, Dh), 0, 2, 1, 3).reshape(B, H, N, L, Dh)
        phi = lambda t: jnp.where(t > 0, t + 1.0, jnp.exp(t))
        scale = Dh ** (-0.5)
        ar = jnp.arange(L)
        mask = (lambda x, dt: x.astype(dt))(ar[:, None] < ar[None, :], x.dtype) * -1000000000.0
        g = _sigmoid(beta).reshape(1, H, 1, 1)
        M = jnp.einsum('bhd,bhe->bhde', q[:, :, 0, 0, :] * 0.0, q[:, :, 0, 0, :] * 0.0)
        z = q[:, :, 0, 0, :] * 0.0
        outs = []
        for s in range(N):
            qs, ks, vs = (q[:, :, s].copy(), k[:, :, s].copy(), v[:, :, s].copy())
            logits = jnp.einsum('bhqd,bhkd->bhqk', qs, ks) * scale + mask
            p = _softmax(logits, axis=-1)
            a_dot = jnp.einsum('bhqk,bhkd->bhqd', p, vs)
            pq = phi(qs)
            num = jnp.einsum('bhld,bhde->bhle', pq, M)
            den = jnp.einsum('bhld,bhd->bhl', pq, z)[..., None] + 1e-06
            a_mem = num / den
            o = g * a_mem + (1.0 - g) * a_dot
            outs.append(o)
            pk = phi(ks)
            M = M + jnp.einsum('bhld,bhle->bhde', pk, vs)
            z = z + jnp.einsum('bhld->bhd', pk)
        o = (lambda x, *d: x.transpose(*d))(jnp.stack(outs, 2).reshape(B, H, S, Dh), 0, 2, 1, 3).reshape(B, S, D)
        return o @ wo

    def _B_ref(x, w1, w2, w3, w4):
        B, S, D = x.shape
        h = _gelu(_layernorm(x, axis=-1) @ w1)
        c = D // 4
        g0 = jnp.pad(h[:, :, 0 * c:1 * c], ((0, 0), (1, 0), (0, 0)))[:, :S, :]
        g1 = jnp.pad(h[:, :, 1 * c:2 * c], ((0, 0), (0, 1), (0, 0)))[:, 1:, :]
        g2 = jnp.pad(h[:, :, 2 * c:3 * c], ((0, 0), (2, 0), (0, 0)))[:, :S, :]
        g3 = jnp.pad(h[:, :, 3 * c:], ((0, 0), (0, 2), (0, 0)))[:, 2:, :]
        hs = jnp.concatenate([g0, g1, g2, g3], axis=-1) @ w2
        x1 = x + hs
        h2 = _gelu(_layernorm(x1, axis=-1) @ w3) @ w4
        return x1 + h2
    x = A_x
    x = x + _A_ref(_layernorm(x, axis=-1), A_wq, A_wk, A_wv, A_wo, A_beta)
    x = x + _B_ref(_layernorm(x, axis=-1), B_w1, B_w2, B_w3, B_w4)
    x = x + _A_ref(_layernorm(x, axis=-1), A_wq, A_wk, A_wv, A_wo, A_beta)
    x = x + _B_ref(_layernorm(x, axis=-1), B_w1, B_w2, B_w3, B_w4)
    return x
```

```python
import functools
import math
import jax
import jax.numpy as jnp
from jax import lax
import jax.experimental.pallas as pl
import jax.experimental.pallas.tpu as pltpu

S, D, F, H, DH, NSEG, L = 2048, 1024, 3584, 32, 32, 4, 512
EPS = 1e-5
NG = D // 128
NT = (((1,), (1,)), ((), ()))
BF = jnp.bfloat16
F32 = jnp.float32
QSCALE = (DH ** -0.5) * math.log2(math.e)
TMA = 512
TMB = 256


def _ln(x):
    m = jnp.mean(x, axis=-1, keepdims=True)
    xc = x - m
    v = jnp.mean(xc * xc, axis=-1, keepdims=True)
    return xc * lax.rsqrt(v + EPS), v


def _gelu(x):
    c = math.sqrt(2.0 / math.pi)
    inner = c * (x + 0.044715 * (x * x * x))
    return 0.5 * x * (1.0 + jnp.tanh(inner))


def _phi(t):
    return jnp.where(t > 0, t + 1.0, jnp.exp(t))


def _dot(a, b):
    return jnp.dot(a, b, preferred_element_type=F32)


def _dot_nt(a, b):
    return lax.dot_general(a, b, NT, preferred_element_type=F32)


def _kernel(x_hbm, wq_hbm, wk_hbm, wv_hbm, wo_hbm, beta_ref, w1_hbm, w2_hbm, w3_hbm, w4_hbm,
            out_hbm,
            XB, X, Y, Wq, Wk, Wv, WvT, Wo, W1, W2, W3, W4,
            Q, PQ, K, PK, VT, O, Hb, MT, ZR, G, sems, osem):
    def cp(src, dst, i):
        return pltpu.make_async_copy(src, dst, sems.at[i])
    xcp = [cp(x_hbm.at[pl.ds(s * L, L)], XB.at[pl.ds(s * L, L)], s) for s in range(NSEG)]
    wcp = [cp(src, dst, 4 + i) for i, (src, dst) in enumerate(
        [(wq_hbm, Wq), (wk_hbm, Wk), (wv_hbm, Wv), (wo_hbm, Wo), (w1_hbm, W1), (w2_hbm, W2), (w3_hbm, W3), (w4_hbm, W4)])]
    xcp[0].start()
    wcp[0].start()
    wcp[1].start()
    wcp[2].start()
    for s in range(1, NSEG):
        xcp[s].start()
    for i in range(3, 8):
        wcp[i].start()

    Hb[pl.ds(0, 8), :] = jnp.zeros((8, D), F32)
    Hb[pl.ds(S + 8, 8), :] = jnp.zeros((8, D), F32)
    b = jax.nn.sigmoid(beta_ref[...].astype(F32))
    rhead = lax.broadcasted_iota(jnp.int32, (D, H), 0) // DH
    chead = lax.broadcasted_iota(jnp.int32, (D, H), 1)
    gcol = jnp.sum(jnp.where(rhead == chead, b, 0.0), axis=1, keepdims=True)
    G[...] = jnp.broadcast_to(gcol, (D, 128))

    for s in range(NSEG):
        xcp[s].wait()
    X[...] = XB[...].astype(F32)
    wcp[2].wait()
    for c in range(D // 128):
        WvT[pl.ds(c * 128, 128), :] = Wv[:, pl.ds(c * 128, 128)].T
    for i in [0, 1, 3, 4, 5, 6, 7]:
        wcp[i].wait()

    lane_head = lax.broadcasted_iota(jnp.int32, (128, 128), 1) // DH
    row_i = lax.broadcasted_iota(jnp.int32, (128, 128), 0)
    col_i = lax.broadcasted_iota(jnp.int32, (128, 128), 1)
    diag_blk = (row_i // DH) == (col_i // DH)

    def qkv_body(i, c):
        r0 = pl.multiple_of(i * TMA, TMA)
        xn, _ = _ln(X[pl.ds(r0, TMA), :])
        xn = xn.astype(BF)
        q = _dot(xn, Wq[...])
        Q[pl.ds(r0, TMA), :] = (q * QSCALE).astype(BF)
        PQ[pl.ds(r0, TMA), :] = _phi(q).astype(BF)
        k = _dot(xn, Wk[...])
        K[pl.ds(r0, TMA), :] = k.astype(BF)
        PK[pl.ds(r0, TMA), :] = _phi(k).astype(BF)
        VT[:, pl.ds(r0, TMA)] = _dot_nt(WvT[...], xn).astype(BF)
        return c

    def attn_body(idx, c):
        s = idx // NG
        g = idx % NG
        r0 = pl.multiple_of(s * L, L)
        c0 = pl.multiple_of(g * 128, 128)

        @pl.when(s == 0)
        def _():
            MT[g] = jnp.zeros((128, 128), F32)
            ZR[g] = jnp.zeros((16, 128), F32)

        Kg = K[pl.ds(r0, L), pl.ds(c0, 128)]
        VTg = VT[pl.ds(c0, 128), pl.ds(r0, L)]
        ones = jnp.ones((16, L), BF)
        lhs = jnp.concatenate([MT[g], ZR[g]], axis=0).astype(BF)
        nd = _dot_nt(lhs, PQ[pl.ds(r0, L), pl.ds(c0, 128)])
        rden = 1.0 / (nd[128:136] + 1e-6)
        gt = G[pl.ds(c0, 128), :]
        gt = jnp.concatenate([gt] * 4, axis=1)
        rden_b = jnp.concatenate(
            [jnp.broadcast_to(rden[h:h + 1], (DH, L)) for h in range(4)], axis=0)
        amem = gt * (nd[:128] * rden_b)

        cols = []
        for j in range(4):
            nk = 128 * (j + 1)
            qj = Q[pl.ds(r0 + 128 * j, 128), pl.ds(c0, 128)]
            qm = jnp.concatenate(
                [jnp.where(lane_head == h, qj, jnp.zeros((), BF)) for h in range(4)], axis=0)
            st = _dot_nt(Kg[:nk], qm)
            causal = jnp.concatenate([row_i <= col_i] * 4, axis=1)
            dg = jnp.where(causal, st[nk - 128:], -1e30)
            st = dg if j == 0 else jnp.concatenate([st[:nk - 128], dg], axis=0)
            m = jnp.max(st, axis=0, keepdims=True)
            p = jnp.exp2(st - m).astype(BF)
            heads = []
            for h in range(4):
                lv = jnp.concatenate([VTg[DH * h:DH * (h + 1), :nk], ones[:, :nk]], axis=0)
                ol = _dot(lv, p[:, 128 * h:128 * (h + 1)])
                heads.append(ol[:DH] * (1.0 / ol[DH:DH + 1]))
            cols.append(jnp.concatenate(heads, axis=0))
        adot = jnp.concatenate(cols, axis=1)
        ot = amem + (1.0 - gt) * adot
        O[pl.ds(r0, L), pl.ds(c0, 128)] = ot.T.astype(BF)

        @pl.when(s < NSEG - 1)
        def _():
            upd = _dot(jnp.concatenate([VTg, ones], axis=0), PK[pl.ds(r0, L), pl.ds(c0, 128)])
            MT[g] += jnp.where(diag_blk, upd[:128], 0.0)
            zrow = upd[128:136]
            hrow = lax.broadcasted_iota(jnp.int32, (8, 128), 0)
            hl = lax.broadcasted_iota(jnp.int32, (8, 128), 1) // DH
            ZR[g, pl.ds(0, 8), :] += jnp.where(hrow == hl, zrow, 0.0)
        return c

    def oproj_body(i, c):
        r0 = pl.multiple_of(i * TMA, TMA)
        x = X[pl.ds(r0, TMA), :] + _dot(O[pl.ds(r0, TMA), :], Wo[...])
        X[pl.ds(r0, TMA), :] = x
        y, v = _ln(x)
        Y[pl.ds(r0, TMA), :] = y
        z = y * lax.rsqrt(v / (v + EPS) + EPS)
        h = _gelu(_dot(z.astype(BF), W1[...]))
        Hb[pl.ds(r0 + 8, TMA), :] = h
        return c

    def mlp_body(i, layer):
        r0 = pl.multiple_of(i * TMB, TMB)
        cw = D // 4
        hb = Hb[pl.ds(r0, TMB + 16), :]
        hs = jnp.concatenate([
            hb[7:7 + TMB, 0 * cw:1 * cw],
            hb[9:9 + TMB, 1 * cw:2 * cw],
            hb[6:6 + TMB, 2 * cw:3 * cw],
            hb[10:10 + TMB, 3 * cw:4 * cw]], axis=1).astype(BF)
        x1 = Y[pl.ds(r0, TMB), :] + _dot(hs, W2[...])
        z1, _ = _ln(x1)
        t = _gelu(_dot(z1.astype(BF), W3[...])).astype(BF)
        xn = X[pl.ds(r0, TMB), :] + x1 + _dot(t, W4[...])
        X[pl.ds(r0, TMB), :] = xn
        O[pl.ds(r0, TMB), :] = xn.astype(BF)

        @pl.when(layer == 1)
        def _():
            pltpu.make_async_copy(O.at[pl.ds(r0, TMB)], out_hbm.at[pl.ds(r0, TMB)], osem.at[i]).start()
        return layer

    def layer_body(layer, c):
        with jax.named_scope("qkv"):
            lax.fori_loop(0, S // TMA, qkv_body, 0)
        with jax.named_scope("attn"):
            lax.fori_loop(0, NSEG * NG, attn_body, 0)
        with jax.named_scope("oproj"):
            lax.fori_loop(0, S // TMA, oproj_body, 0)
        with jax.named_scope("mlp"):
            lax.fori_loop(0, S // TMB, mlp_body, layer)
        return c

    lax.fori_loop(0, 2, layer_body, 0)
    for i in range(S // TMB):
        pltpu.make_async_copy(O.at[pl.ds(i * TMB, TMB)], out_hbm.at[pl.ds(i * TMB, TMB)], osem.at[i]).wait()


@jax.jit
def pallas_interleave_layers__memory_aug_infini_attn__mixer_s_mlp__prompt_kernel(A_x, A_wq, A_wk, A_wv, A_wo, A_beta, B_x, B_w1, B_w2, B_w3, B_w4):
    anyspec = pl.BlockSpec(memory_space=pl.ANY)
    out = pl.pallas_call(
        _kernel,
        out_shape=jax.ShapeDtypeStruct((S, D), BF),
        in_specs=[anyspec] * 5 + [pl.BlockSpec(memory_space=pltpu.VMEM)] + [anyspec] * 4,
        out_specs=anyspec,
        scratch_shapes=[
            pltpu.VMEM((S, D), BF),
            pltpu.VMEM((S, D), F32),
            pltpu.VMEM((S, D), F32),
            pltpu.VMEM((D, D), BF), pltpu.VMEM((D, D), BF), pltpu.VMEM((D, D), BF),
            pltpu.VMEM((D, D), BF),
            pltpu.VMEM((D, D), BF), pltpu.VMEM((D, D), BF), pltpu.VMEM((D, D), BF),
            pltpu.VMEM((D, F), BF), pltpu.VMEM((F, D), BF),
            pltpu.VMEM((S, D), BF), pltpu.VMEM((S, D), BF), pltpu.VMEM((S, D), BF), pltpu.VMEM((S, D), BF),
            pltpu.VMEM((D, S), BF),
            pltpu.VMEM((S, D), BF),
            pltpu.VMEM((S + 16, D), F32),
            pltpu.VMEM((NG, 128, 128), F32),
            pltpu.VMEM((NG, 16, 128), F32),
            pltpu.VMEM((D, 128), F32),
            pltpu.SemaphoreType.DMA((12,)),
            pltpu.SemaphoreType.DMA((S // TMB,)),
        ],
        compiler_params=pltpu.CompilerParams(vmem_limit_bytes=120 * 1024 * 1024),
    )(A_x.reshape(S, D), A_wq, A_wk, A_wv, A_wo, A_beta.reshape(1, H), B_w1, B_w2, B_w3, B_w4)
    return out.reshape(1, S, D)
```

```python
import functools
import math
import jax
import jax.numpy as jnp
from jax import lax
import jax.experimental.pallas as pl
import jax.experimental.pallas.tpu as pltpu

S, D, F, H, DH, NSEG, L = 2048, 1024, 3584, 32, 32, 4, 512
EPS = 1e-5
NG = D // 128
NT = (((1,), (1,)), ((), ()))
BF = jnp.bfloat16
F32 = jnp.float32
I32 = jnp.int32
QSCALE = (DH ** -0.5) * math.log2(math.e)
TMA = 512
TMB = 256
L_LO = 2.0 ** -60
ACC_HI_BITS = (127 + 100) << 23


def _ln(x):
    m = jnp.mean(x, axis=-1, keepdims=True)
    xc = x - m
    v = jnp.mean(xc * xc, axis=-1, keepdims=True)
    return xc * lax.rsqrt(v + EPS), v


def _gelu(x):
    c = math.sqrt(2.0 / math.pi)
    inner = c * (x + 0.044715 * (x * x * x))
    return 0.5 * x * (1.0 + jnp.tanh(inner))


def _phi(t):
    return jnp.where(t > 0, t + 1.0, jnp.exp(t))


def _dot(a, b):
    return jnp.dot(a, b, preferred_element_type=F32)


def _dot_nt(a, b):
    return lax.dot_general(a, b, NT, preferred_element_type=F32)


def _pk(x):
    return pltpu.bitcast(x, I32)


def _up(x):
    return pltpu.bitcast(x, BF)


def _kernel(x_hbm, wq_hbm, wk_hbm, wv_hbm, wo_hbm, beta_ref, w1_hbm, w2_hbm, w3_hbm, w4_hbm,
            out_hbm,
            XB, X, Y, Wq, Wk, Wv, WvT, Wo, W1, W2, W3, W4,
            Q, PQ, K, PK, VT, O, Hb, MT, ZR, G, sems, osem):
    def cp(src, dst, i):
        return pltpu.make_async_copy(src, dst, sems.at[i])
    xcp = [cp(x_hbm.at[pl.ds(s * L, L)], XB.at[pl.ds(s * L, L)], s) for s in range(NSEG)]
    wcp = [cp(src, dst, 4 + i) for i, (src, dst) in enumerate(
        [(wv_hbm, Wv), (wq_hbm, Wq), (wk_hbm, Wk), (wo_hbm, Wo), (w1_hbm, W1), (w2_hbm, W2), (w3_hbm, W3), (w4_hbm, W4)])]
    wcp[0].start()
    xcp[0].start()
    wcp[1].start()
    wcp[2].start()

    Hb[pl.ds(0, 8), :] = jnp.zeros((8, D), F32)
    Hb[pl.ds(S + 8, 8), :] = jnp.zeros((8, D), F32)
    b = jax.nn.sigmoid(beta_ref[...].astype(F32))
    rhead = lax.broadcasted_iota(jnp.int32, (D, H), 0) // DH
    chead = lax.broadcasted_iota(jnp.int32, (D, H), 1)
    gcol = jnp.sum(jnp.where(rhead == chead, b, 0.0), axis=1, keepdims=True)
    G[...] = jnp.broadcast_to(gcol, (D, 128))

    wcp[0].wait()
    for c in range(D // 128):
        WvT[pl.ds(c * 128, 128), :] = Wv[:, pl.ds(c * 128, 128)].T
    xcp[0].wait()
    for s in range(1, NSEG):
        xcp[s].start()
    X[pl.ds(0, L), :] = XB[pl.ds(0, L), :].astype(F32)
    wcp[1].wait()
    wcp[2].wait()
    for i in range(3, 8):
        wcp[i].start()
    for s in range(1, NSEG):
        xcp[s].wait()
        X[pl.ds(s * L, L), :] = XB[pl.ds(s * L, L), :].astype(F32)

    def qkv_body(i, c):
        r0 = pl.multiple_of(i * TMA, TMA)
        h0 = pl.multiple_of(i * (TMA // 2), TMA // 2)
        xn, _ = _ln(X[pl.ds(r0, TMA), :])
        xn = xn.astype(BF)
        q = _dot(xn, Wq[...])
        Q[pl.ds(h0, TMA // 2), :] = _pk((q * QSCALE).astype(BF))
        PQ[pl.ds(h0, TMA // 2), :] = _pk(_phi(q).astype(BF))
        k = _dot(xn, Wk[...])
        K[pl.ds(h0, TMA // 2), :] = _pk(k.astype(BF))
        PK[pl.ds(h0, TMA // 2), :] = _pk(_phi(k).astype(BF))
        VT[:, pl.ds(r0, TMA)] = _pk(_dot_nt(WvT[...], xn).astype(BF))
        return c

    def consts():
        lane_head = lax.broadcasted_iota(jnp.int32, (64, 128), 1) // DH
        row_i = lax.broadcasted_iota(jnp.int32, (128, 128), 0)
        col_i = lax.broadcasted_iota(jnp.int32, (128, 128), 1)
        causal = jnp.concatenate([row_i <= col_i] * 4, axis=1)
        diag_blk = (row_i // DH) == (col_i // DH)
        zmask = lax.broadcasted_iota(jnp.int32, (8, 128), 0) == lax.broadcasted_iota(jnp.int32, (8, 128), 1) // DH
        return lane_head, causal, diag_blk, zmask

    def scores(cs, h0, c0, j):
        lane_head, causal, _, _ = cs
        qj = Q[pl.ds(h0 + 64 * j, 64), pl.ds(c0, 128)]
        qm = _up(jnp.concatenate([jnp.where(lane_head == h, qj, 0) for h in range(4)], axis=0))
        kk = _up(K[pl.ds(h0, 64 * (j + 1)), pl.ds(c0, 128)])
        st = _dot_nt(kk, qm)
        tiles = [st[128 * t:128 * (t + 1)] for t in range(j + 1)]
        tiles[j] = jnp.where(causal, tiles[j], -1e30)
        return tiles

    def pv(tiles, m, e0, r0):
        ones = jnp.ones((16, 128), BF)
        acc = [None] * 4
        for t, tile in enumerate(tiles):
            for h in range(4):
                x = tile[:, 128 * h:128 * (h + 1)]
                if m is not None:
                    x = x - m[:, 128 * h:128 * (h + 1)]
                p = jnp.exp2(x).astype(BF)
                lv = jnp.concatenate([_up(VT[pl.ds(e0 + 16 * h, 16), pl.ds(r0 + 128 * t, 128)]), ones], axis=0)
                ol = _dot(lv, p)[:DH + 8]
                acc[h] = ol if t == 0 else acc[h] + ol
        return acc

    def mem_read(mt, zr, h0, c0):
        lhs = jnp.concatenate([mt, zr, jnp.zeros((8, 128), F32)], axis=0).astype(BF)
        nd = _dot_nt(lhs, _up(PQ[pl.ds(h0, L // 2), pl.ds(c0, 128)]))
        rden = 1.0 / (nd[128:136] + 1e-6)
        rden_b = jnp.concatenate([jnp.broadcast_to(rden[h:h + 1], (DH, L)) for h in range(4)], axis=0)
        return nd[:128] * rden_b

    def mem_update(cs, mt, zr, h0, c0, e0, r0):
        _, _, diag_blk, zmask = cs
        vg = _up(VT[pl.ds(e0, 64), pl.ds(r0, L)])
        upd = _dot(jnp.concatenate([vg, jnp.ones((16, L), BF)], axis=0), _up(PK[pl.ds(h0, L // 2), pl.ds(c0, 128)]))
        dm = jnp.where(diag_blk, upd[:128], 0.0)
        dz = jnp.where(zmask, upd[128:136], 0.0)
        return (dm, dz) if mt is None else (mt + dm, zr + dz)

    def store_o(ot, h0, c0, j):
        O[pl.ds(h0 + 64 * j, 64), pl.ds(c0, 128)] = _pk(ot.T.astype(BF))

    def attn_fast(g, carry):
        lmin, amax = carry
        cs = consts()
        c0 = pl.multiple_of(g * 128, 128)
        e0 = pl.multiple_of(g * 64, 64)
        gt = G[pl.ds(c0, 128), :]
        mt = zr = None
        for s in range(NSEG):
            r0, h0 = s * L, s * (L // 2)
            cols = {}
            for j in (3, 2, 1, 0):
                tl = scores(cs, h0, c0, j)
                if j == 0 and s > 0:
                    amem = mem_read(mt, zr, h0, c0)
                acc = pv(tl, None, e0, r0)
                for a in acc:
                    lmin = jnp.minimum(lmin, a[DH:])
                    ab = pltpu.bitcast(a, I32) & 0x7FFFFFFF
                    for r in range(5):
                        amax = jnp.maximum(amax, ab[8 * r:8 * r + 8])
                cols[j] = jnp.concatenate([a[:DH] * (1.0 / a[DH:DH + 1]) for a in acc], axis=0)
            for j in range(4):
                if s > 0:
                    ot = gt * amem[:, 128 * j:128 * (j + 1)] + (1.0 - gt) * cols[j]
                else:
                    ot = (1.0 - gt) * cols[j]
                store_o(ot, h0, c0, j)
            if s < NSEG - 1:
                mt, zr = mem_update(cs, mt, zr, h0, c0, e0, r0)
        return lmin, amax

    def attn_exact(idx, c):
        s = idx // NG
        g = idx % NG
        cs = consts()
        r0 = pl.multiple_of(s * L, L)
        h0 = pl.multiple_of(s * (L // 2), L // 2)
        c0 = pl.multiple_of(g * 128, 128)
        e0 = pl.multiple_of(g * 64, 64)
        gt = G[pl.ds(c0, 128), :]
        amem = mem_read(MT[g], ZR[g], h0, c0)
        for j in range(4):
            tl = scores(cs, h0, c0, j)
            mx = tl[0]
            for t in tl[1:]:
                mx = jnp.maximum(mx, t)
            m = jnp.max(mx, axis=0, keepdims=True)
            acc = pv(tl, m, e0, r0)
            col = jnp.concatenate([a[:DH] * (1.0 / a[DH:DH + 1]) for a in acc], axis=0)
            store_o(gt * amem[:, 128 * j:128 * (j + 1)] + (1.0 - gt) * col, h0, c0, j)
        MT[g], ZR[g] = mem_update(cs, MT[g], ZR[g], h0, c0, e0, r0)
        return c

    def attn_phase():
        lmin, amax = lax.fori_loop(0, NG, attn_fast,
                                   (jnp.full((8, 128), 1.0, F32), jnp.zeros((8, 128), I32)))
        safe = jnp.logical_and(jnp.min(lmin) >= L_LO, jnp.max(amax) <= ACC_HI_BITS)

        @pl.when(jnp.logical_not(safe))
        def _():
            MT[...] = jnp.zeros((NG, 128, 128), F32)
            ZR[...] = jnp.zeros((NG, 8, 128), F32)
            lax.fori_loop(0, NSEG * NG, attn_exact, 0)

    def oproj_body(i, c):
        r0 = pl.multiple_of(i * TMA, TMA)
        h0 = pl.multiple_of(i * (TMA // 2), TMA // 2)
        x = X[pl.ds(r0, TMA), :] + _dot(_up(O[pl.ds(h0, TMA // 2), :]), Wo[...])
        X[pl.ds(r0, TMA), :] = x
        y, v = _ln(x)
        Y[pl.ds(r0, TMA), :] = y
        z = y * lax.rsqrt(v / (v + EPS) + EPS)
        h = _gelu(_dot(z.astype(BF), W1[...]))
        Hb[pl.ds(r0 + 8, TMA), :] = h
        return c

    def mlp_body(i, layer):
        r0 = pl.multiple_of(i * TMB, TMB)
        cw = D // 4
        hb = Hb[pl.ds(r0, TMB + 16), :]
        hs = jnp.concatenate([
            hb[7:7 + TMB, 0 * cw:1 * cw],
            hb[9:9 + TMB, 1 * cw:2 * cw],
            hb[6:6 + TMB, 2 * cw:3 * cw],
            hb[10:10 + TMB, 3 * cw:4 * cw]], axis=1).astype(BF)
        x1 = Y[pl.ds(r0, TMB), :] + _dot(hs, W2[...])
        z1, _ = _ln(x1)
        t = _gelu(_dot(z1.astype(BF), W3[...])).astype(BF)
        xn = X[pl.ds(r0, TMB), :] + x1 + _dot(t, W4[...])
        X[pl.ds(r0, TMB), :] = xn
        XB[pl.ds(r0, TMB), :] = xn.astype(BF)

        @pl.when(layer == 1)
        def _():
            pltpu.make_async_copy(XB.at[pl.ds(r0, TMB)], out_hbm.at[pl.ds(r0, TMB)], osem.at[i]).start()
        return layer

    def layer_body(layer, c):
        with jax.named_scope("qkv"):
            lax.fori_loop(0, S // TMA, qkv_body, 0)
        with jax.named_scope("attn"):
            attn_phase()

        @pl.when(layer == 0)
        def _():
            for i in range(3, 8):
                wcp[i].wait()
        with jax.named_scope("oproj"):
            lax.fori_loop(0, S // TMA, oproj_body, 0)
        with jax.named_scope("mlp"):
            lax.fori_loop(0, S // TMB, mlp_body, layer)
        return c

    lax.fori_loop(0, 2, layer_body, 0)
    for i in range(S // TMB):
        pltpu.make_async_copy(XB.at[pl.ds(i * TMB, TMB)], out_hbm.at[pl.ds(i * TMB, TMB)], osem.at[i]).wait()


@jax.jit
def pallas_interleave_layers__memory_aug_infini_attn__mixer_s_mlp__prompt_kernel(A_x, A_wq, A_wk, A_wv, A_wo, A_beta, B_x, B_w1, B_w2, B_w3, B_w4):
    anyspec = pl.BlockSpec(memory_space=pl.ANY)
    out = pl.pallas_call(
        _kernel,
        out_shape=jax.ShapeDtypeStruct((S, D), BF),
        in_specs=[anyspec] * 5 + [pl.BlockSpec(memory_space=pltpu.VMEM)] + [anyspec] * 4,
        out_specs=anyspec,
        scratch_shapes=[
            pltpu.VMEM((S, D), BF),
            pltpu.VMEM((S, D), F32),
            pltpu.VMEM((S, D), F32),
            pltpu.VMEM((D, D), BF), pltpu.VMEM((D, D), BF), pltpu.VMEM((D, D), BF),
            pltpu.VMEM((D, D), BF),
            pltpu.VMEM((D, D), BF), pltpu.VMEM((D, D), BF), pltpu.VMEM((D, D), BF),
            pltpu.VMEM((D, F), BF), pltpu.VMEM((F, D), BF),
            pltpu.VMEM((S // 2, D), I32), pltpu.VMEM((S // 2, D), I32),
            pltpu.VMEM((S // 2, D), I32), pltpu.VMEM((S // 2, D), I32),
            pltpu.VMEM((D // 2, S), I32),
            pltpu.VMEM((S // 2, D), I32),
            pltpu.VMEM((S + 16, D), F32),
            pltpu.VMEM((NG, 128, 128), F32),
            pltpu.VMEM((NG, 8, 128), F32),
            pltpu.VMEM((D, 128), F32),
            pltpu.SemaphoreType.DMA((12,)),
            pltpu.SemaphoreType.DMA((S // TMB,)),
        ],
        compiler_params=pltpu.CompilerParams(vmem_limit_bytes=120 * 1024 * 1024),
    )(A_x.reshape(S, D), A_wq, A_wk, A_wv, A_wo, A_beta.reshape(1, H), B_w1, B_w2, B_w3, B_w4)
    return out.reshape(1, S, D)
```

```python
import functools
import math
import jax
import jax.numpy as jnp
from jax import lax
import jax.experimental.pallas as pl
import jax.experimental.pallas.tpu as pltpu

S, D, F, H, DH, NSEG, L = 2048, 1024, 3584, 32, 32, 4, 512
EPS = 1e-5
NG = D // 128
NT = (((1,), (1,)), ((), ()))
BF = jnp.bfloat16
F32 = jnp.float32
I32 = jnp.int32
QSCALE = (DH ** -0.5) * math.log2(math.e)
TMA = 512
TMB = 256
TS = 256
L_LO = 2.0 ** -60
ACC_HI_BITS = (127 + 100) << 23


def _ln(x):
    m = jnp.mean(x, axis=-1, keepdims=True)
    xc = x - m
    v = jnp.mean(xc * xc, axis=-1, keepdims=True)
    return xc * lax.rsqrt(v + EPS), v


def _gelu(x):
    c = math.sqrt(2.0 / math.pi)
    inner = c * (x + 0.044715 * (x * x * x))
    return 0.5 * x * (1.0 + jnp.tanh(inner))


def _phi(t):
    return jnp.where(t > 0, t + 1.0, jnp.exp(t))


def _dot(a, b):
    return jnp.dot(a, b, preferred_element_type=F32)


def _dot_nt(a, b):
    return lax.dot_general(a, b, NT, preferred_element_type=F32)


def _pk(x):
    return pltpu.bitcast(x, I32)


def _up(x):
    return pltpu.bitcast(x, BF)


def _acombos(a):
    m2, k2 = a.shape[0] // 2, a.shape[1] // 2
    a11, a12, a21, a22 = a[:m2, :k2], a[:m2, k2:], a[m2:, :k2], a[m2:, k2:]
    return [x.astype(BF) for x in (a11 + a22, a21 + a22, a11, a22, a11 + a12, a21 - a11, a12 - a22)]


def _sdot(ac, Wp):
    m1, m2, m3, m4, m5, m6, m7 = [_dot(ac[i], Wp[i]) for i in range(7)]
    c11 = m1 + m4 - m5 + m7
    c12 = m3 + m5
    c21 = m2 + m4
    c22 = m1 - m2 + m3 + m6
    return jnp.concatenate([jnp.concatenate([c11, c12], 1), jnp.concatenate([c21, c22], 1)], 0)


def _prep(Wp, rows):
    b11 = Wp[1, rows, :].astype(F32)
    b12 = Wp[2, rows, :].astype(F32)
    b21 = Wp[3, rows, :].astype(F32)
    b22 = Wp[4, rows, :].astype(F32)
    Wp[0, rows, :] = (b11 + b22).astype(BF)
    Wp[2, rows, :] = (b12 - b22).astype(BF)
    Wp[3, rows, :] = (b21 - b11).astype(BF)
    Wp[5, rows, :] = (b11 + b12).astype(BF)
    Wp[6, rows, :] = (b21 + b22).astype(BF)


def _prep_all(Wp, step=64):
    n = Wp.shape[1] // step
    def body(i, c):
        _prep(Wp, pl.ds(pl.multiple_of(i * step, step), step))
        return c
    lax.fori_loop(0, n, body, 0)


def _kernel(x_hbm, wq_hbm, wk_hbm, wv_hbm, wo_hbm, beta_ref, w1_hbm, w2_hbm, w3_hbm, w4_hbm,
            out_hbm,
            XB, X, Y, Wq, Wk, Wv, Wo, W1, W2, W3, W4,
            Q, PQ, K, PK, VT, O, Hb, MT, ZR, G, sems, osem):
    def cp(src, dst, i):
        return pltpu.make_async_copy(src, dst, sems.at[i])
    xcp = [cp(x_hbm.at[pl.ds(s * L, L)], XB.at[pl.ds(s * L, L)], s) for s in range(NSEG)]
    def wcps(src, dst, i):
        k2, n2 = src.shape[0] // 2, src.shape[1] // 2
        return [cp(src.at[pl.ds(a * k2, k2), pl.ds(b * n2, n2)], dst.at[1 + 2 * a + b], 4 + 4 * i + 2 * a + b)
                for a in (0, 1) for b in (0, 1)]
    wcp = [wcps(src, dst, i) for i, (src, dst) in enumerate(
        [(wq_hbm, Wq), (wk_hbm, Wk), (wv_hbm, Wv), (wo_hbm, Wo), (w1_hbm, W1), (w2_hbm, W2), (w3_hbm, W3), (w4_hbm, W4)])]

    def start(i):
        for c in wcp[i]:
            c.start()

    def wait(i):
        for c in wcp[i]:
            c.wait()
    xcp[0].start()
    start(0)
    start(1)
    start(2)

    Hb[pl.ds(0, 8), :] = jnp.zeros((8, D), F32)
    Hb[pl.ds(S + 8, 8), :] = jnp.zeros((8, D), F32)
    b = jax.nn.sigmoid(beta_ref[...].astype(F32))
    rhead = lax.broadcasted_iota(jnp.int32, (D, H), 0) // DH
    chead = lax.broadcasted_iota(jnp.int32, (D, H), 1)
    gcol = jnp.sum(jnp.where(rhead == chead, b, 0.0), axis=1, keepdims=True)
    G[...] = jnp.broadcast_to(gcol, (D, 128))

    xcp[0].wait()
    for s in range(1, NSEG):
        xcp[s].start()
    X[pl.ds(0, L), :] = XB[pl.ds(0, L), :].astype(F32)
    wait(0)
    _prep_all(Wq)
    wait(1)
    _prep_all(Wk)
    wait(2)
    for i in range(3, 8):
        start(i)
    _prep_all(Wv)
    for s in range(1, NSEG):
        xcp[s].wait()
        X[pl.ds(s * L, L), :] = XB[pl.ds(s * L, L), :].astype(F32)

    def qkv_body(i, c):
        for u in range(TMA // TS):
            r0 = pl.multiple_of(i * TMA + u * TS, TS)
            h0 = pl.multiple_of(i * (TMA // 2) + u * (TS // 2), TS // 2)
            xn, _ = _ln(X[pl.ds(r0, TS), :])
            ac = _acombos(xn)
            q = _sdot(ac, Wq)
            Q[pl.ds(h0, TS // 2), :] = _pk((q * QSCALE).astype(BF))
            PQ[pl.ds(h0, TS // 2), :] = _pk(_phi(q).astype(BF))
            k = _sdot(ac, Wk)
            K[pl.ds(h0, TS // 2), :] = _pk(k.astype(BF))
            PK[pl.ds(h0, TS // 2), :] = _pk(_phi(k).astype(BF))
            v = _sdot(ac, Wv)
            VT[:, pl.ds(r0, TS)] = _pk(v.T.astype(BF))
        return c

    def consts():
        lane_head = lax.broadcasted_iota(jnp.int32, (64, 128), 1) // DH
        row_i = lax.broadcasted_iota(jnp.int32, (128, 128), 0)
        col_i = lax.broadcasted_iota(jnp.int32, (128, 128), 1)
        causal = jnp.concatenate([row_i <= col_i] * 4, axis=1)
        diag_blk = (row_i // DH) == (col_i // DH)
        zmask = lax.broadcasted_iota(jnp.int32, (8, 128), 0) == lax.broadcasted_iota(jnp.int32, (8, 128), 1) // DH
        return lane_head, causal, diag_blk, zmask

    def scores(cs, h0, c0, j):
        lane_head, causal, _, _ = cs
        qj = Q[pl.ds(h0 + 64 * j, 64), pl.ds(c0, 128)]
        qm = _up(jnp.concatenate([jnp.where(lane_head == h, qj, 0) for h in range(4)], axis=0))
        kk = _up(K[pl.ds(h0, 64 * (j + 1)), pl.ds(c0, 128)])
        st = _dot_nt(kk, qm)
        tiles = [st[128 * t:128 * (t + 1)] for t in range(j + 1)]
        tiles[j] = jnp.where(causal, tiles[j], -1e30)
        return tiles

    def pv(tiles, m, e0, r0):
        ones = jnp.ones((16, 128), BF)
        acc = [None] * 4
        for t, tile in enumerate(tiles):
            for h in range(4):
                x = tile[:, 128 * h:128 * (h + 1)]
                if m is not None:
                    x = x - m[:, 128 * h:128 * (h + 1)]
                p = jnp.exp2(x).astype(BF)
                lv = jnp.concatenate([_up(VT[pl.ds(e0 + 16 * h, 16), pl.ds(r0 + 128 * t, 128)]), ones], axis=0)
                ol = _dot(lv, p)[:DH + 8]
                acc[h] = ol if t == 0 else acc[h] + ol
        return acc

    def mem_read(mt, zr, h0, c0):
        lhs = jnp.concatenate([mt, zr, jnp.zeros((8, 128), F32)], axis=0).astype(BF)
        nd = _dot_nt(lhs, _up(PQ[pl.ds(h0, L // 2), pl.ds(c0, 128)]))
        rden = 1.0 / (nd[128:136] + 1e-6)
        rden_b = jnp.concatenate([jnp.broadcast_to(rden[h:h + 1], (DH, L)) for h in range(4)], axis=0)
        return nd[:128] * rden_b

    def mem_update(cs, mt, zr, h0, c0, e0, r0):
        _, _, diag_blk, zmask = cs
        vg = _up(VT[pl.ds(e0, 64), pl.ds(r0, L)])
        upd = _dot(jnp.concatenate([vg, jnp.ones((16, L), BF)], axis=0), _up(PK[pl.ds(h0, L // 2), pl.ds(c0, 128)]))
        dm = jnp.where(diag_blk, upd[:128], 0.0)
        dz = jnp.where(zmask, upd[128:136], 0.0)
        return (dm, dz) if mt is None else (mt + dm, zr + dz)

    def store_o(ot, h0, c0, j):
        O[pl.ds(h0 + 64 * j, 64), pl.ds(c0, 128)] = _pk(ot.T.astype(BF))

    def attn_fast(g, carry):
        lmin, amax = carry
        cs = consts()
        c0 = pl.multiple_of(g * 128, 128)
        e0 = pl.multiple_of(g * 64, 64)
        gt = G[pl.ds(c0, 128), :]
        mt = zr = None
        for s in range(NSEG):
            r0, h0 = s * L, s * (L // 2)
            cols = {}
            for j in (3, 2, 1, 0):
                tl = scores(cs, h0, c0, j)
                if j == 0 and s > 0:
                    amem = mem_read(mt, zr, h0, c0)
                acc = pv(tl, None, e0, r0)
                for a in acc:
                    lmin = jnp.minimum(lmin, a[DH:])
                    ab = pltpu.bitcast(a, I32) & 0x7FFFFFFF
                    for r in range(5):
                        amax = jnp.maximum(amax, ab[8 * r:8 * r + 8])
                cols[j] = jnp.concatenate([a[:DH] * (1.0 / a[DH:DH + 1]) for a in acc], axis=0)
            for j in range(4):
                if s > 0:
                    ot = gt * amem[:, 128 * j:128 * (j + 1)] + (1.0 - gt) * cols[j]
                else:
                    ot = (1.0 - gt) * cols[j]
                store_o(ot, h0, c0, j)
            if s < NSEG - 1:
                mt, zr = mem_update(cs, mt, zr, h0, c0, e0, r0)
        return lmin, amax

    def attn_exact(idx, c):
        s = idx // NG
        g = idx % NG
        cs = consts()
        r0 = pl.multiple_of(s * L, L)
        h0 = pl.multiple_of(s * (L // 2), L // 2)
        c0 = pl.multiple_of(g * 128, 128)
        e0 = pl.multiple_of(g * 64, 64)
        gt = G[pl.ds(c0, 128), :]
        amem = mem_read(MT[g], ZR[g], h0, c0)
        for j in range(4):
            tl = scores(cs, h0, c0, j)
            mx = tl[0]
            for t in tl[1:]:
                mx = jnp.maximum(mx, t)
            m = jnp.max(mx, axis=0, keepdims=True)
            acc = pv(tl, m, e0, r0)
            col = jnp.concatenate([a[:DH] * (1.0 / a[DH:DH + 1]) for a in acc], axis=0)
            store_o(gt * amem[:, 128 * j:128 * (j + 1)] + (1.0 - gt) * col, h0, c0, j)
        MT[g], ZR[g] = mem_update(cs, MT[g], ZR[g], h0, c0, e0, r0)
        return c

    def attn_phase():
        lmin, amax = lax.fori_loop(0, NG, attn_fast,
                                   (jnp.full((8, 128), 1.0, F32), jnp.zeros((8, 128), I32)))
        safe = jnp.logical_and(jnp.min(lmin) >= L_LO, jnp.max(amax) <= ACC_HI_BITS)

        @pl.when(jnp.logical_not(safe))
        def _():
            MT[...] = jnp.zeros((NG, 128, 128), F32)
            ZR[...] = jnp.zeros((NG, 8, 128), F32)
            lax.fori_loop(0, NSEG * NG, attn_exact, 0)

    def oproj_body(i, c):
        nsub = TMA // TS
        r0s = [pl.multiple_of(i * TMA + u * TS, TS) for u in range(nsub)]
        h0s = [pl.multiple_of(i * (TMA // 2) + u * (TS // 2), TS // 2) for u in range(nsub)]
        xs = []
        for u in range(nsub):
            o = _up(O[pl.ds(h0s[u], TS // 2), :]).astype(F32)
            x = X[pl.ds(r0s[u], TS), :] + _sdot(_acombos(o), Wo)
            X[pl.ds(r0s[u], TS), :] = x
            xs.append(x)
        for u in range(nsub):
            y, v = _ln(xs[u])
            Y[pl.ds(r0s[u], TS), :] = y
            z = y * lax.rsqrt(v / (v + EPS) + EPS)
            h = _gelu(_sdot(_acombos(z), W1))
            Hb[pl.ds(r0s[u] + 8, TS), :] = h
        return c

    def mlp_body(i, layer):
        nsub = TMB // TS
        r0s = [pl.multiple_of(i * TMB + u * TS, TS) for u in range(nsub)]
        cw = D // 4
        x1s = []
        for u in range(nsub):
            hb = Hb[pl.ds(r0s[u], TS + 16), :]
            hs = jnp.concatenate([
                hb[7:7 + TS, 0 * cw:1 * cw],
                hb[9:9 + TS, 1 * cw:2 * cw],
                hb[6:6 + TS, 2 * cw:3 * cw],
                hb[10:10 + TS, 3 * cw:4 * cw]], axis=1)
            x1s.append(Y[pl.ds(r0s[u], TS), :] + _sdot(_acombos(hs), W2))
        ts = []
        for u in range(nsub):
            z1, _ = _ln(x1s[u])
            ts.append(_gelu(_sdot(_acombos(z1), W3)))
        for u in range(nsub):
            xn = X[pl.ds(r0s[u], TS), :] + x1s[u] + _sdot(_acombos(ts[u]), W4)
            X[pl.ds(r0s[u], TS), :] = xn
            XB[pl.ds(r0s[u], TS), :] = xn.astype(BF)
        r0 = pl.multiple_of(i * TMB, TMB)

        @pl.when(layer == 1)
        def _():
            pltpu.make_async_copy(XB.at[pl.ds(r0, TMB)], out_hbm.at[pl.ds(r0, TMB)], osem.at[i]).start()
        return layer

    def layer_body(layer, c):
        with jax.named_scope("qkv"):
            lax.fori_loop(0, S // TMA, qkv_body, 0)
        with jax.named_scope("attn"):
            attn_phase()

        @pl.when(layer == 0)
        def _():
            for i in range(3, 8):
                wait(i)
            for w in (Wo, W1, W2, W3, W4):
                _prep_all(w)
        with jax.named_scope("oproj"):
            lax.fori_loop(0, S // TMA, oproj_body, 0)
        with jax.named_scope("mlp"):
            lax.fori_loop(0, S // TMB, mlp_body, layer)
        return c

    lax.fori_loop(0, 2, layer_body, 0)
    for i in range(S // TMB):
        pltpu.make_async_copy(XB.at[pl.ds(i * TMB, TMB)], out_hbm.at[pl.ds(i * TMB, TMB)], osem.at[i]).wait()


@jax.jit
def pallas_interleave_layers__memory_aug_infini_attn__mixer_s_mlp__prompt_kernel(A_x, A_wq, A_wk, A_wv, A_wo, A_beta, B_x, B_w1, B_w2, B_w3, B_w4):
    anyspec = pl.BlockSpec(memory_space=pl.ANY)
    out = pl.pallas_call(
        _kernel,
        out_shape=jax.ShapeDtypeStruct((S, D), BF),
        in_specs=[anyspec] * 5 + [pl.BlockSpec(memory_space=pltpu.VMEM)] + [anyspec] * 4,
        out_specs=anyspec,
        scratch_shapes=[
            pltpu.VMEM((S, D), BF),
            pltpu.VMEM((S, D), F32),
            pltpu.VMEM((S, D), F32),
            *[pltpu.VMEM((7, D // 2, D // 2), BF)] * 6,
            pltpu.VMEM((7, D // 2, F // 2), BF), pltpu.VMEM((7, F // 2, D // 2), BF),
            pltpu.VMEM((S // 2, D), I32), pltpu.VMEM((S // 2, D), I32),
            pltpu.VMEM((S // 2, D), I32), pltpu.VMEM((S // 2, D), I32),
            pltpu.VMEM((D // 2, S), I32),
            pltpu.VMEM((S // 2, D), I32),
            pltpu.VMEM((S + 16, D), F32),
            pltpu.VMEM((NG, 128, 128), F32),
            pltpu.VMEM((NG, 8, 128), F32),
            pltpu.VMEM((D, 128), F32),
            pltpu.SemaphoreType.DMA((36,)),
            pltpu.SemaphoreType.DMA((S // TMB,)),
        ],
        compiler_params=pltpu.CompilerParams(vmem_limit_bytes=120 * 1024 * 1024),
    )(A_x.reshape(S, D), A_wq, A_wk, A_wv, A_wo, A_beta.reshape(1, H), B_w1, B_w2, B_w3, B_w4)
    return out.reshape(1, S, D)
```

```python
import math
import jax
import jax.numpy as jnp
from jax import lax
import jax.experimental.pallas as pl
import jax.experimental.pallas.tpu as pltpu

S, D, F, H, DH, NSEG, L = 2048, 1024, 3584, 32, 32, 4, 512
EPS = 1e-5
NG = D // 128
NT = (((1,), (1,)), ((), ()))
BF = jnp.bfloat16
F32 = jnp.float32
I32 = jnp.int32
QSCALE = (DH ** -0.5) * math.log2(math.e)
TM = 512
NB = S // TM
L_LO = 2.0 ** -60
ACC_HI_BITS = (127 + 100) << 23
LV_SMALL = 2
LV_BIG = 2
ORDER = (2, 4, 3, 1, 0, 5, 6)

A_Q, A_PQ, A_K, A_PK, A_VT = (i * (S // 2) for i in range(5))
A_H = 0
A_T = (0, 1024, 2048, 3072)
ARENA = 5 * (S // 2)


def _ln(x):
    m = jnp.mean(x, axis=-1, keepdims=True)
    xc = x - m
    v = jnp.mean(xc * xc, axis=-1, keepdims=True)
    return xc * lax.rsqrt(v + EPS), v


def _gelu(x):
    c = math.sqrt(2.0 / math.pi)
    inner = c * (x + 0.044715 * (x * x * x))
    return 0.5 * x * (1.0 + jnp.tanh(inner))


def _phi(t):
    return jnp.where(t > 0, t + 1.0, jnp.exp(t))


def _dot(a, b):
    return jnp.dot(a, b, preferred_element_type=F32)


def _dot_nt(a, b):
    return lax.dot_general(a, b, NT, preferred_element_type=F32)


def _pk(x):
    return pltpu.bitcast(x, I32)


def _up(x):
    return pltpu.bitcast(x, BF)


def _quad(a):
    m2, k2 = a.shape[0] // 2, a.shape[1] // 2
    return a[:m2, :k2], a[:m2, k2:], a[m2:, :k2], a[m2:, k2:]


def _left(a11, a12, a21, a22):
    return (a11 + a22, a21 + a22, a11, a22, a11 + a12, a21 - a11, a12 - a22)


def _right(b11, b12, b21, b22):
    return (b11 + b22, b11, b12 - b22, b21 - b11, b22, b11 + b12, b21 + b22)


def _acombos(a, level):
    if level == 0:
        return a.astype(BF)
    return [_acombos(x, level - 1) for x in _left(*_quad(a))]


class _Filler:
    def __init__(self, jobs=(), slots=1):
        self.jobs, self.slots, self.calls, self.done = list(jobs), slots, 0, 0

    def __call__(self):
        self.calls += 1
        while self.done < len(self.jobs) and self.done * self.slots < self.calls * len(self.jobs):
            self.jobs[self.done]()
            self.done += 1


def _sdot(ac, Wp, level, fill=None, base=0):
    if level == 0:
        out = _dot(ac, _up(Wp[base]))
        if fill is not None:
            fill()
        return out
    m = [None] * 7
    for i in ORDER:
        m[i] = _sdot(ac[i], Wp, level - 1, fill, base * 7 + i)
    m1, m2, m3, m4, m5, m6, m7 = m
    c11 = m1 + m4 - m5 + m7
    c12 = m3 + m5
    c21 = m2 + m4
    c22 = m1 - m2 + m3 + m6
    return jnp.concatenate([jnp.concatenate([c11, c12], 1), jnp.concatenate([c21, c22], 1)], 0)


def _raw_slots(level):
    out = [(0, 0, 0)]
    for _ in range(level):
        out = [(7 * s + 1 + 2 * a + b, 2 * r + a, 2 * c + b) for (s, r, c) in out for a in (0, 1) for b in (0, 1)]
    return out


def _prep(Wp, level, rows):
    for c0 in range(0, Wp.shape[2], 128):
        _prep_strip(Wp, level, rows, pl.ds(c0, 128))


def _prep_strip(Wp, level, rows, cols):
    raw = {(r, c): (s, _up(Wp[s, rows, cols])) for (s, r, c) in _raw_slots(level)}
    outs = []

    def rec(blk, lv, base):
        if lv == 0:
            slot, val = blk[(0, 0)]
            if slot != base:
                outs.append((base, _pk(val.astype(BF))))
            return
        hh = 2 ** (lv - 1)
        cells = [(r, c) for r in range(hh) for c in range(hh)]
        quads = [{rc: blk[(rc[0] + a * hh, rc[1] + b * hh)] for rc in cells} for a in (0, 1) for b in (0, 1)]
        for i in range(7):
            if i == 1:
                sub = quads[0]
            elif i == 4:
                sub = quads[3]
            else:
                sub = {rc: (None, _right(*[q[rc][1].astype(F32) for q in quads])[i]) for rc in cells}
            rec(sub, lv - 1, base * 7 + i)
            if lv == 1:
                pass
        if lv == 1 and level > 1:
            flush()

    def flush():
        for base, val in outs:
            Wp[base, rows, cols] = val
        outs.clear()
    rec(raw, level, 0)
    flush()


def _prep_loop(Wp, level, step=8):
    def body(i, c):
        _prep(Wp, level, pl.ds(pl.multiple_of(i * step, step), step))
        return c
    lax.fori_loop(0, Wp.shape[1] // step, body, 0)


def _kernel(x_hbm, wq_hbm, wk_hbm, wv_hbm, wo_hbm, beta_ref, w1_hbm, w2_hbm, w3_hbm, w4_hbm,
            out_hbm,
            X, Wq, Wk, Wv, Wo, W1, W2, W3, W4, A, O, MT, ZR, G, xsem, wsem, osem):
    x32 = x_hbm.bitcast(I32)
    out32 = out_hbm.bitcast(I32)
    xcp = [pltpu.make_async_copy(x32.at[pl.ds(s * L // 2, L // 2)], O.at[pl.ds(s * L // 2, L // 2)], xsem.at[s])
           for s in range(NSEG)]

    def wcps(src, dst, level, i):
        kb, nb = dst.shape[1], dst.shape[2]
        src = src.bitcast(I32)
        return [pltpu.make_async_copy(src.at[pl.ds(r * kb, kb), pl.ds(c * nb, nb)], dst.at[s], wsem.at[i])
                for (s, r, c) in _raw_slots(level)]
    weights = [(wq_hbm, Wq, LV_SMALL), (wk_hbm, Wk, LV_SMALL), (wv_hbm, Wv, LV_SMALL), (wo_hbm, Wo, LV_SMALL),
               (w1_hbm, W1, LV_SMALL), (w2_hbm, W2, LV_SMALL), (w3_hbm, W3, LV_BIG), (w4_hbm, W4, LV_BIG)]
    wcp = [wcps(src, dst, lv, i) for i, (src, dst, lv) in enumerate(weights)]

    def start(i):
        for c in wcp[i]:
            c.start()

    def wait(i):
        for c in wcp[i]:
            c.wait()
    xcp[0].start()
    start(0)
    start(1)
    start(2)

    b = jax.nn.sigmoid(beta_ref[...].astype(F32))
    rhead = lax.broadcasted_iota(jnp.int32, (D, H), 0) // DH
    chead = lax.broadcasted_iota(jnp.int32, (D, H), 1)
    gcol = jnp.sum(jnp.where(rhead == chead, b, 0.0), axis=1, keepdims=True)
    G[...] = jnp.broadcast_to(gcol, (D, 128))

    xcp[0].wait()
    for s in range(1, NSEG):
        xcp[s].start()
    X[pl.ds(0, L), :] = _up(O[pl.ds(0, L // 2), :]).astype(F32)
    wait(0)
    _prep_loop(Wq, LV_SMALL)
    wait(1)
    _prep_loop(Wk, LV_SMALL)
    wait(2)
    for i in range(3, 8):
        start(i)
    _prep_loop(Wv, LV_SMALL)
    for s in range(1, NSEG):
        xcp[s].wait()
        X[pl.ds(s * L, L), :] = _up(O[pl.ds(s * L // 2, L // 2), :]).astype(F32)

    def prep_jobs(Wp, lv, i, n, strips):
        return [(lambda u=u, c=c: _prep_strip(Wp, lv, pl.ds(pl.multiple_of((i * n + u) * 8, 8), 8), pl.ds(128 * c, 128)))
                for u in range(n) for c in strips]

    def rows(i):
        return pl.multiple_of(i * TM, TM), pl.multiple_of(i * (TM // 2), TM // 2)

    def qkv_body(i, c):
        r0, h0 = rows(i)
        xn, _ = _ln(X[pl.ds(r0, TM), :])
        ac = _acombos(xn, LV_SMALL)
        q = _sdot(ac, Wq, LV_SMALL)
        A[pl.ds(A_Q + h0, TM // 2), :] = _pk((q * QSCALE).astype(BF))
        A[pl.ds(A_PQ + h0, TM // 2), :] = _pk(_phi(q).astype(BF))
        k = _sdot(ac, Wk, LV_SMALL)
        A[pl.ds(A_K + h0, TM // 2), :] = _pk(k.astype(BF))
        A[pl.ds(A_PK + h0, TM // 2), :] = _pk(_phi(k).astype(BF))
        v = _sdot(ac, Wv, LV_SMALL)
        vr = pl.multiple_of(A_VT + (i // 2) * (D // 2), D // 2)
        vc = pl.multiple_of((i % 2) * TM, TM)
        A[pl.ds(vr, D // 2), pl.ds(vc, TM)] = _pk(v.T.astype(BF))
        return c

    def consts():
        lane_head = lax.broadcasted_iota(jnp.int32, (64, 128), 1) // DH
        row_i = lax.broadcasted_iota(jnp.int32, (128, 128), 0)
        col_i = lax.broadcasted_iota(jnp.int32, (128, 128), 1)
        causal = jnp.concatenate([row_i <= col_i] * 4, axis=1)
        diag_blk = (row_i // DH) == (col_i // DH)
        zmask = lax.broadcasted_iota(jnp.int32, (8, 128), 0) == lax.broadcasted_iota(jnp.int32, (8, 128), 1) // DH
        return lane_head, causal, diag_blk, zmask

    def vt(e0, n_e, r0, n_k):
        if isinstance(r0, int):
            return _up(A[pl.ds(A_VT + (r0 // D) * (D // 2) + e0, n_e), pl.ds(r0 % D, n_k)])
        vr = pl.multiple_of(A_VT + (r0 // D) * (D // 2) + e0, 16)
        return _up(A[pl.ds(vr, n_e), pl.ds(pl.multiple_of(r0 % D, 128), n_k)])

    def scores(cs, h0, c0, j):
        lane_head, causal, _, _ = cs
        qj = A[pl.ds(A_Q + h0 + 64 * j, 64), pl.ds(c0, 128)]
        qm = _up(jnp.concatenate([jnp.where(lane_head == h, qj, 0) for h in range(4)], axis=0))
        kk = _up(A[pl.ds(A_K + h0, 64 * (j + 1)), pl.ds(c0, 128)])
        st = _dot_nt(kk, qm)
        tiles = [st[128 * t:128 * (t + 1)] for t in range(j + 1)]
        tiles[j] = jnp.where(causal, tiles[j], -1e30)
        return tiles

    def pv(tiles, m, e0, r0):
        ones = jnp.ones((16, 128), BF)
        acc = [None] * 4
        for t, tile in enumerate(tiles):
            for h in range(4):
                x = tile[:, 128 * h:128 * (h + 1)]
                if m is not None:
                    x = x - m[:, 128 * h:128 * (h + 1)]
                p = jnp.exp2(x).astype(BF)
                lv = jnp.concatenate([vt(e0 + 16 * h, 16, r0 + 128 * t, 128), ones], axis=0)
                ol = _dot(lv, p)[:DH + 8]
                acc[h] = ol if t == 0 else acc[h] + ol
        return acc

    def mem_read(mt, zr, h0, c0):
        lhs = jnp.concatenate([mt, zr, jnp.zeros((8, 128), F32)], axis=0).astype(BF)
        nd = _dot_nt(lhs, _up(A[pl.ds(A_PQ + h0, L // 2), pl.ds(c0, 128)]))
        rden = 1.0 / (nd[128:136] + 1e-6)
        rden_b = jnp.concatenate([jnp.broadcast_to(rden[h:h + 1], (DH, L)) for h in range(4)], axis=0)
        return nd[:128] * rden_b

    def mem_update(cs, mt, zr, h0, c0, e0, r0):
        _, _, diag_blk, zmask = cs
        vg = vt(e0, 64, r0, L)
        upd = _dot(jnp.concatenate([vg, jnp.ones((16, L), BF)], axis=0),
                   _up(A[pl.ds(A_PK + h0, L // 2), pl.ds(c0, 128)]))
        dm = jnp.where(diag_blk, upd[:128], 0.0)
        dz = jnp.where(zmask, upd[128:136], 0.0)
        return (dm, dz) if mt is None else (mt + dm, zr + dz)

    def store_o(ot, h0, c0, j):
        O[pl.ds(h0 + 64 * j, 64), pl.ds(c0, 128)] = _pk(ot.T.astype(BF))

    def attn_fast(g, carry, prep):
        lmin, amax = carry
        cs = consts()
        c0 = pl.multiple_of(g * 128, 128)
        e0 = pl.multiple_of(g * 64, 64)
        gt = G[pl.ds(c0, 128), :]
        mt = zr = None
        fill = _Filler()
        if prep:
            fill = _Filler(prep_jobs(Wo, LV_SMALL, g, 2, range(2)) + prep_jobs(W3, LV_BIG, g, 2, range(4)), 16)
        for s in range(NSEG):
            r0, h0 = s * L, s * (L // 2)
            cols = {}
            for j in (3, 2, 1, 0):
                tl = scores(cs, h0, c0, j)
                if j == 0 and s > 0:
                    amem = mem_read(mt, zr, h0, c0)
                acc = pv(tl, None, e0, r0)
                fill()
                for a in acc:
                    lmin = jnp.minimum(lmin, a[DH:])
                    ab = pltpu.bitcast(a, I32) & 0x7FFFFFFF
                    for r in range(5):
                        amax = jnp.maximum(amax, ab[8 * r:8 * r + 8])
                cols[j] = jnp.concatenate([a[:DH] * (1.0 / a[DH:DH + 1]) for a in acc], axis=0)
            for j in range(4):
                if s > 0:
                    ot = gt * amem[:, 128 * j:128 * (j + 1)] + (1.0 - gt) * cols[j]
                else:
                    ot = (1.0 - gt) * cols[j]
                store_o(ot, h0, c0, j)
            if s < NSEG - 1:
                mt, zr = mem_update(cs, mt, zr, h0, c0, e0, r0)
        return lmin, amax

    def attn_exact(idx, c):
        s = idx // NG
        g = idx % NG
        cs = consts()
        r0 = pl.multiple_of(s * L, L)
        h0 = pl.multiple_of(s * (L // 2), L // 2)
        c0 = pl.multiple_of(g * 128, 128)
        e0 = pl.multiple_of(g * 64, 64)
        gt = G[pl.ds(c0, 128), :]
        amem = mem_read(MT[g], ZR[g], h0, c0)
        for j in range(4):
            tl = scores(cs, h0, c0, j)
            mx = tl[0]
            for t in tl[1:]:
                mx = jnp.maximum(mx, t)
            m = jnp.max(mx, axis=0, keepdims=True)
            acc = pv(tl, m, e0, r0)
            col = jnp.concatenate([a[:DH] * (1.0 / a[DH:DH + 1]) for a in acc], axis=0)
            store_o(gt * amem[:, 128 * j:128 * (j + 1)] + (1.0 - gt) * col, h0, c0, j)
        MT[g], ZR[g] = mem_update(cs, MT[g], ZR[g], h0, c0, e0, r0)
        return c

    def attn_phase(prep):
        lmin, amax = lax.fori_loop(0, NG, lambda g, carry: attn_fast(g, carry, prep),
                                   (jnp.full((8, 128), 1.0, F32), jnp.zeros((8, 128), I32)))
        safe = jnp.logical_and(jnp.min(lmin) >= L_LO, jnp.max(amax) <= ACC_HI_BITS)

        @pl.when(jnp.logical_not(safe))
        def _():
            MT[...] = jnp.zeros((NG, 128, 128), F32)
            ZR[...] = jnp.zeros((NG, 8, 128), F32)
            lax.fori_loop(0, NSEG * NG, attn_exact, 0)

    def oproj_body(i, c, prep):
        r0, h0 = rows(i)
        fill = _Filler(prep_jobs(W1, LV_SMALL, i, 4, range(2)) + prep_jobs(W3, LV_BIG, i, 4, [4]), 40) if prep else None
        o = _up(O[pl.ds(h0, TM // 2), :]).astype(F32)
        x = X[pl.ds(r0, TM), :] + _sdot(_acombos(o, LV_SMALL), Wo, LV_SMALL, fill)
        X[pl.ds(r0, TM), :] = x
        return c

    def w1_body(i, c, prep):
        r0, h0 = rows(i)
        fill = _Filler(prep_jobs(W2, LV_SMALL, i, 4, range(2)), 40) if prep else None
        y, v = _ln(X[pl.ds(r0, TM), :])
        z = y * lax.rsqrt(v / (v + EPS) + EPS)
        h = _gelu(_sdot(_acombos(z, LV_SMALL), W1, LV_SMALL, fill))
        A[pl.ds(A_H + 8 + r0, TM), :] = pltpu.bitcast(h, I32)
        return c

    def w2_body(i, c, prep):
        r0, h0 = rows(i)
        fill = _Filler(prep_jobs(W3, LV_BIG, i, 4, [5, 6]), 40) if prep else None
        cw = D // 4
        hb = pltpu.bitcast(A[pl.ds(A_H + r0, TM + 16), :], F32)
        hs = jnp.concatenate([
            hb[7:7 + TM, 0 * cw:1 * cw],
            hb[9:9 + TM, 1 * cw:2 * cw],
            hb[6:6 + TM, 2 * cw:3 * cw],
            hb[10:10 + TM, 3 * cw:4 * cw]], axis=1)
        x = X[pl.ds(r0, TM), :]
        y, _ = _ln(x)
        x1 = y + _sdot(_acombos(hs, LV_SMALL), W2, LV_SMALL, fill)
        X[pl.ds(r0, TM), :] = x + x1
        z1, _ = _ln(x1)
        O[pl.ds(h0, TM // 2), :] = _pk(z1.astype(BF))
        return c

    def w3_body(i, c, prep):
        r0, h0 = rows(i)
        fill = _Filler(prep_jobs(W4, LV_BIG, i, 14, range(2)), 40) if prep else None
        z1 = _up(O[pl.ds(h0, TM // 2), :]).astype(F32)
        t = _pk(_gelu(_sdot(_acombos(z1, LV_BIG), W3, LV_BIG, fill)).astype(BF))
        fq = F // 4
        for q in range(4):
            A[pl.ds(A_T[q] + h0, TM // 2), pl.ds(0, fq)] = t[:, q * fq:(q + 1) * fq]
        return c

    def w4_body(i, c, last):
        r0, h0 = rows(i)
        fq = F // 4
        t = jnp.concatenate([_up(A[pl.ds(A_T[q] + h0, TM // 2), pl.ds(0, fq)]) for q in range(4)], axis=1).astype(F32)
        xn = X[pl.ds(r0, TM), :] + _sdot(_acombos(t, LV_BIG), W4, LV_BIG)
        if last:
            O[pl.ds(h0, TM // 2), :] = _pk(xn.astype(BF))
            pltpu.make_async_copy(O.at[pl.ds(h0, TM // 2)], out32.at[pl.ds(h0, TM // 2)], osem.at[i]).start()
        else:
            X[pl.ds(r0, TM), :] = xn
        return c

    for layer in range(2):
        with jax.named_scope("qkv"):
            lax.fori_loop(0, NB, qkv_body, 0)
        if layer == 0:
            for i in range(3, 8):
                wait(i)
        with jax.named_scope("attn"):
            attn_phase(layer == 0)
        with jax.named_scope("oproj"):
            lax.fori_loop(0, NB, lambda i, c: oproj_body(i, c, layer == 0), 0)
        A[pl.ds(A_H, 8), :] = jnp.zeros((8, D), I32)
        A[pl.ds(A_H + S + 8, 8), :] = jnp.zeros((8, D), I32)
        with jax.named_scope("w1"):
            lax.fori_loop(0, NB, lambda i, c: w1_body(i, c, layer == 0), 0)
        with jax.named_scope("w2"):
            lax.fori_loop(0, NB, lambda i, c: w2_body(i, c, layer == 0), 0)
        with jax.named_scope("w3"):
            lax.fori_loop(0, NB, lambda i, c: w3_body(i, c, layer == 0), 0)
        with jax.named_scope("w4"):
            lax.fori_loop(0, NB, lambda i, c: w4_body(i, c, layer == 1), 0)
    for i in range(NB):
        pltpu.make_async_copy(O.at[pl.ds(i * TM // 2, TM // 2)], out32.at[pl.ds(i * TM // 2, TM // 2)], osem.at[i]).wait()


def _wshape(k, n, level):
    return pltpu.VMEM((7 ** level, k >> (level + 1), n >> level), I32)


@jax.jit
def pallas_interleave_layers__memory_aug_infini_attn__mixer_s_mlp__prompt_kernel(A_x, A_wq, A_wk, A_wv, A_wo, A_beta, B_x, B_w1, B_w2, B_w3, B_w4):
    anyspec = pl.BlockSpec(memory_space=pl.ANY)
    out = pl.pallas_call(
        _kernel,
        out_shape=jax.ShapeDtypeStruct((S, D), BF),
        in_specs=[anyspec] * 5 + [pl.BlockSpec(memory_space=pltpu.VMEM)] + [anyspec] * 4,
        out_specs=anyspec,
        scratch_shapes=[
            pltpu.VMEM((S, D), F32),
            *[_wshape(D, D, LV_SMALL)] * 6,
            _wshape(D, F, LV_BIG), _wshape(F, D, LV_BIG),
            pltpu.VMEM((ARENA, D), I32),
            pltpu.VMEM((S // 2, D), I32),
            pltpu.VMEM((NG, 128, 128), F32),
            pltpu.VMEM((NG, 8, 128), F32),
            pltpu.VMEM((D, 128), F32),
            pltpu.SemaphoreType.DMA((NSEG,)),
            pltpu.SemaphoreType.DMA((8,)),
            pltpu.SemaphoreType.DMA((NB,)),
        ],
        compiler_params=pltpu.CompilerParams(vmem_limit_bytes=128 * 1024 * 1024),
    )(A_x.reshape(S, D), A_wq, A_wk, A_wv, A_wo, A_beta.reshape(1, H), B_w1, B_w2, B_w3, B_w4)
    return out.reshape(1, S, D)
```

```python
import math
import jax
import jax.numpy as jnp
from jax import lax
import jax.experimental.pallas as pl
import jax.experimental.pallas.tpu as pltpu

S, D, F, H, DH, NSEG, L = 2048, 1024, 3584, 32, 32, 4, 512
EPS = 1e-5
NG = D // 128
NT = (((1,), (1,)), ((), ()))
BF = jnp.bfloat16
F32 = jnp.float32
I32 = jnp.int32
QSCALE = (DH ** -0.5) * math.log2(math.e)
TM = 512
NB = S // TM
L_LO = 2.0 ** -60
ACC_HI_BITS = (127 + 100) << 23
LV_SMALL = 2
LV_BIG = 2
ORDER = (2, 4, 3, 1, 0, 5, 6)

A_Q, A_PQ, A_K, A_PK, A_VT = (i * (S // 2) for i in range(5))
A_H = 0
A_T = (0, 1024, 2048, 3072)
ARENA = 5 * (S // 2)


def _ln(x):
    m = jnp.mean(x, axis=-1, keepdims=True)
    xc = x - m
    v = jnp.mean(xc * xc, axis=-1, keepdims=True)
    return xc * lax.rsqrt(v + EPS), v


def _gelu(x):
    c = math.sqrt(2.0 / math.pi)
    inner = c * (x + 0.044715 * (x * x * x))
    return 0.5 * x * (1.0 + jnp.tanh(inner))


def _phi(t):
    return jnp.where(t > 0, t + 1.0, jnp.exp(t))


def _dot(a, b):
    return jnp.dot(a, b, preferred_element_type=F32)


def _dot_nt(a, b):
    return lax.dot_general(a, b, NT, preferred_element_type=F32)


def _pk(x):
    return pltpu.bitcast(x, I32)


def _up(x):
    return pltpu.bitcast(x, BF)


def _quad(a):
    m2, k2 = a.shape[0] // 2, a.shape[1] // 2
    return a[:m2, :k2], a[:m2, k2:], a[m2:, :k2], a[m2:, k2:]


def _left(a11, a12, a21, a22):
    return (a11 + a22, a21 + a22, a11, a22, a11 + a12, a21 - a11, a12 - a22)


def _right(b11, b12, b21, b22):
    return (b11 + b22, b11, b12 - b22, b21 - b11, b22, b11 + b12, b21 + b22)


def _acombos(a, level):
    if level == 0:
        return a.astype(BF)
    return [_acombos(x, level - 1) for x in _left(*_quad(a))]


class _Filler:
    def __init__(self, jobs=(), slots=1):
        self.jobs, self.slots, self.calls, self.done = list(jobs), slots, 0, 0

    def __call__(self):
        self.calls += 1
        while self.done < len(self.jobs) and self.done * self.slots < self.calls * len(self.jobs):
            self.jobs[self.done]()
            self.done += 1


def _sdot(ac, Wp, level, fill=None, base=0, top=None):
    top = level if top is None else top
    if level == 0:
        out = _dot(ac, _up(Wp[_w(Wp, top, _slot_of_product(top)[base])]))
        if fill is not None:
            fill()
        return out
    m = [None] * 7
    for i in ORDER:
        m[i] = _sdot(ac[i], Wp, level - 1, fill, base * 7 + i, top)
    m1, m2, m3, m4, m5, m6, m7 = m
    c11 = m1 + m4 - m5 + m7
    c12 = m3 + m5
    c21 = m2 + m4
    c22 = m1 - m2 + m3 + m6
    return jnp.concatenate([jnp.concatenate([c11, c12], 1), jnp.concatenate([c21, c22], 1)], 0)


def _raw_slots(level):
    n = 2 ** level
    return [(n * c + r, r, c) for c in range(n) for r in range(n)]


def _slot_of_product(level):
    n = 2 ** level
    asis = [(0, 0)]
    for _ in range(level):
        asis = [(7 * p + i, 2 * d + (i == 4)) for (p, d) in asis for i in (1, 4)]
    table = {p: n * d + d for (p, d) in asis}
    free = [s for s in range(7 ** level) if s not in table.values()]
    for p in range(7 ** level):
        if p not in table:
            table[p] = free.pop(0)
    return table


def _w(Wp, level, slot, rows=None, cols=None):
    kb = Wp.shape[0] // 7 ** level
    r = pl.ds(slot * kb, kb) if rows is None else pl.ds(slot * kb + rows[0], rows[1])
    return (r, slice(None) if cols is None else cols)


def _prep(Wp, level, rows):
    for c0 in range(0, Wp.shape[1], 128):
        _prep_strip(Wp, level, rows, pl.ds(c0, 128))


def _prep_strip(Wp, level, rows, cols):
    raw = {(r, c): (s, _up(Wp[_w(Wp, level, s, rows, cols)])) for (s, r, c) in _raw_slots(level)}
    outs = []

    def rec(blk, lv, base):
        if lv == 0:
            slot, val = blk[(0, 0)]
            if slot is None:
                outs.append((_slot_of_product(level)[base], _pk(val.astype(BF))))
            else:
                assert slot == _slot_of_product(level)[base]
            return
        hh = 2 ** (lv - 1)
        cells = [(r, c) for r in range(hh) for c in range(hh)]
        quads = [{rc: blk[(rc[0] + a * hh, rc[1] + b * hh)] for rc in cells} for a in (0, 1) for b in (0, 1)]
        for i in range(7):
            if i == 1:
                sub = quads[0]
            elif i == 4:
                sub = quads[3]
            else:
                sub = {rc: (None, _right(*[q[rc][1].astype(F32) for q in quads])[i]) for rc in cells}
            rec(sub, lv - 1, base * 7 + i)
            if lv == 1:
                pass
        if lv == 1 and level > 1:
            flush()

    def flush():
        for base, val in outs:
            Wp[_w(Wp, level, base, rows, cols)] = val
        outs.clear()
    rec(raw, level, 0)
    flush()


def _prep_loop(Wp, level, step=8):
    def body(i, c):
        _prep(Wp, level, (pl.multiple_of(i * step, step), step))
        return c
    lax.fori_loop(0, Wp.shape[0] // 7 ** level // step, body, 0)


def _kernel(x_hbm, wq_hbm, wk_hbm, wv_hbm, wo_hbm, beta_ref, w1_hbm, w2_hbm, w3_hbm, w4_hbm,
            out_hbm,
            X, Wq, Wk, Wv, Wo, W1, W2, W3, W4, A, O, MT, ZR, G, xsem, wsem, osem):
    x32 = x_hbm.bitcast(I32)
    out32 = out_hbm.bitcast(I32)
    xcp = [pltpu.make_async_copy(x32.at[pl.ds(s * L // 2, L // 2)], O.at[pl.ds(s * L // 2, L // 2)], xsem.at[s])
           for s in range(NSEG)]

    def wcps(src, dst, level, i):
        n = 2 ** level
        kb, nb = dst.shape[0] // 7 ** level, dst.shape[1]
        src = src.bitcast(I32)
        return [pltpu.make_async_copy(src.at[:, pl.ds(c * nb, nb)], dst.at[pl.ds(n * c * kb, n * kb)], wsem.at[i])
                for c in range(n)]
    weights = [(wq_hbm, Wq, LV_SMALL), (wk_hbm, Wk, LV_SMALL), (wv_hbm, Wv, LV_SMALL), (wo_hbm, Wo, LV_SMALL),
               (w1_hbm, W1, LV_SMALL), (w2_hbm, W2, LV_SMALL), (w3_hbm, W3, LV_BIG), (w4_hbm, W4, LV_BIG)]
    wcp = [wcps(src, dst, lv, i) for i, (src, dst, lv) in enumerate(weights)]

    def start(i):
        for c in wcp[i]:
            c.start()

    def wait(i):
        for c in wcp[i]:
            c.wait()
    xcp[0].start()
    start(0)

    b = jax.nn.sigmoid(beta_ref[...].astype(F32))
    rhead = lax.broadcasted_iota(jnp.int32, (D, H), 0) // DH
    chead = lax.broadcasted_iota(jnp.int32, (D, H), 1)
    gcol = jnp.sum(jnp.where(rhead == chead, b, 0.0), axis=1, keepdims=True)
    G[...] = jnp.broadcast_to(gcol, (D, 128))

    xcp[0].wait()
    start(1)
    X[pl.ds(0, L), :] = _up(O[pl.ds(0, L // 2), :]).astype(F32)
    wait(0)
    start(2)
    _prep_loop(Wq, LV_SMALL)
    wait(1)
    for s in range(1, NSEG):
        xcp[s].start()
    _prep_loop(Wk, LV_SMALL)
    wait(2)
    for i in range(3, 8):
        start(i)
    _prep_loop(Wv, LV_SMALL)
    for s in range(1, NSEG):
        xcp[s].wait()
        X[pl.ds(s * L, L), :] = _up(O[pl.ds(s * L // 2, L // 2), :]).astype(F32)

    def prep_jobs(Wp, lv, i, n, strips):
        return [(lambda u=u, c=c: _prep_strip(Wp, lv, (pl.multiple_of((i * n + u) * 8, 8), 8), pl.ds(128 * c, 128)))
                for u in range(n) for c in strips]

    def rows(i):
        return pl.multiple_of(i * TM, TM), pl.multiple_of(i * (TM // 2), TM // 2)

    def qkv_body(i, c):
        r0, h0 = rows(i)
        xn, _ = _ln(X[pl.ds(r0, TM), :])
        ac = _acombos(xn, LV_SMALL)
        q = _sdot(ac, Wq, LV_SMALL)
        A[pl.ds(A_Q + h0, TM // 2), :] = _pk((q * QSCALE).astype(BF))
        A[pl.ds(A_PQ + h0, TM // 2), :] = _pk(_phi(q).astype(BF))
        k = _sdot(ac, Wk, LV_SMALL)
        A[pl.ds(A_K + h0, TM // 2), :] = _pk(k.astype(BF))
        A[pl.ds(A_PK + h0, TM // 2), :] = _pk(_phi(k).astype(BF))
        v = _sdot(ac, Wv, LV_SMALL)
        vr = pl.multiple_of(A_VT + (i // 2) * (D // 2), D // 2)
        vc = pl.multiple_of((i % 2) * TM, TM)
        A[pl.ds(vr, D // 2), pl.ds(vc, TM)] = _pk(v.T.astype(BF))
        return c

    def consts():
        lane_head = lax.broadcasted_iota(jnp.int32, (64, 128), 1) // DH
        row_i = lax.broadcasted_iota(jnp.int32, (128, 128), 0)
        col_i = lax.broadcasted_iota(jnp.int32, (128, 128), 1)
        causal = jnp.concatenate([row_i <= col_i] * 4, axis=1)
        diag_blk = (row_i // DH) == (col_i // DH)
        zmask = lax.broadcasted_iota(jnp.int32, (8, 128), 0) == lax.broadcasted_iota(jnp.int32, (8, 128), 1) // DH
        return lane_head, causal, diag_blk, zmask

    def vt(e0, n_e, r0, n_k):
        if isinstance(r0, int):
            return _up(A[pl.ds(A_VT + (r0 // D) * (D // 2) + e0, n_e), pl.ds(r0 % D, n_k)])
        vr = pl.multiple_of(A_VT + (r0 // D) * (D // 2) + e0, 16)
        return _up(A[pl.ds(vr, n_e), pl.ds(pl.multiple_of(r0 % D, 128), n_k)])

    def scores(cs, h0, c0, j):
        lane_head, causal, _, _ = cs
        qj = A[pl.ds(A_Q + h0 + 64 * j, 64), pl.ds(c0, 128)]
        qm = _up(jnp.concatenate([jnp.where(lane_head == h, qj, 0) for h in range(4)], axis=0))
        kk = _up(A[pl.ds(A_K + h0, 64 * (j + 1)), pl.ds(c0, 128)])
        st = _dot_nt(kk, qm)
        tiles = [st[128 * t:128 * (t + 1)] for t in range(j + 1)]
        tiles[j] = jnp.where(causal, tiles[j], -1e30)
        return tiles

    def pv(tiles, m, e0, r0):
        ones = jnp.ones((16, 128), BF)
        acc = [None] * 4
        for t, tile in enumerate(tiles):
            for h in range(4):
                x = tile[:, 128 * h:128 * (h + 1)]
                if m is not None:
                    x = x - m[:, 128 * h:128 * (h + 1)]
                p = jnp.exp2(x).astype(BF)
                lv = jnp.concatenate([vt(e0 + 16 * h, 16, r0 + 128 * t, 128), ones], axis=0)
                ol = _dot(lv, p)[:DH + 8]
                acc[h] = ol if t == 0 else acc[h] + ol
        return acc

    def mem_read(mt, zr, h0, c0):
        lhs = jnp.concatenate([mt, zr, jnp.zeros((8, 128), F32)], axis=0).astype(BF)
        nd = _dot_nt(lhs, _up(A[pl.ds(A_PQ + h0, L // 2), pl.ds(c0, 128)]))
        rden = 1.0 / (nd[128:136] + 1e-6)
        rden_b = jnp.concatenate([jnp.broadcast_to(rden[h:h + 1], (DH, L)) for h in range(4)], axis=0)
        return nd[:128] * rden_b

    def mem_update(cs, mt, zr, h0, c0, e0, r0):
        _, _, diag_blk, zmask = cs
        vg = vt(e0, 64, r0, L)
        upd = _dot(jnp.concatenate([vg, jnp.ones((16, L), BF)], axis=0),
                   _up(A[pl.ds(A_PK + h0, L // 2), pl.ds(c0, 128)]))
        dm = jnp.where(diag_blk, upd[:128], 0.0)
        dz = jnp.where(zmask, upd[128:136], 0.0)
        return (dm, dz) if mt is None else (mt + dm, zr + dz)

    def store_o(ot, h0, c0, j):
        O[pl.ds(h0 + 64 * j, 64), pl.ds(c0, 128)] = _pk(ot.T.astype(BF))

    def attn_fast(g, carry, prep):
        lmin, amax = carry
        cs = consts()
        c0 = pl.multiple_of(g * 128, 128)
        e0 = pl.multiple_of(g * 64, 64)
        gt = G[pl.ds(c0, 128), :]
        mt = zr = None
        fill = _Filler()
        if prep:
            fill = _Filler(prep_jobs(Wo, LV_SMALL, g, 2, range(2)) + prep_jobs(W3, LV_BIG, g, 2, range(4)), 16)
        for s in range(NSEG):
            r0, h0 = s * L, s * (L // 2)
            cols = {}
            for j in (3, 2, 1, 0):
                tl = scores(cs, h0, c0, j)
                if j == 0 and s > 0:
                    amem = mem_read(mt, zr, h0, c0)
                acc = pv(tl, None, e0, r0)
                fill()
                for a in acc:
                    lmin = jnp.minimum(lmin, a[DH:])
                    ab = pltpu.bitcast(a, I32) & 0x7FFFFFFF
                    for r in range(5):
                        amax = jnp.maximum(amax, ab[8 * r:8 * r + 8])
                cols[j] = jnp.concatenate([a[:DH] * (1.0 / a[DH:DH + 1]) for a in acc], axis=0)
            for j in range(4):
                if s > 0:
                    ot = gt * amem[:, 128 * j:128 * (j + 1)] + (1.0 - gt) * cols[j]
                else:
                    ot = (1.0 - gt) * cols[j]
                store_o(ot, h0, c0, j)
            if s < NSEG - 1:
                mt, zr = mem_update(cs, mt, zr, h0, c0, e0, r0)
        return lmin, amax

    def attn_exact(idx, c):
        s = idx // NG
        g = idx % NG
        cs = consts()
        r0 = pl.multiple_of(s * L, L)
        h0 = pl.multiple_of(s * (L // 2), L // 2)
        c0 = pl.multiple_of(g * 128, 128)
        e0 = pl.multiple_of(g * 64, 64)
        gt = G[pl.ds(c0, 128), :]
        amem = mem_read(MT[g], ZR[g], h0, c0)
        for j in range(4):
            tl = scores(cs, h0, c0, j)
            mx = tl[0]
            for t in tl[1:]:
                mx = jnp.maximum(mx, t)
            m = jnp.max(mx, axis=0, keepdims=True)
            acc = pv(tl, m, e0, r0)
            col = jnp.concatenate([a[:DH] * (1.0 / a[DH:DH + 1]) for a in acc], axis=0)
            store_o(gt * amem[:, 128 * j:128 * (j + 1)] + (1.0 - gt) * col, h0, c0, j)
        MT[g], ZR[g] = mem_update(cs, MT[g], ZR[g], h0, c0, e0, r0)
        return c

    def attn_phase(prep):
        lmin, amax = lax.fori_loop(0, NG, lambda g, carry: attn_fast(g, carry, prep),
                                   (jnp.full((8, 128), 1.0, F32), jnp.zeros((8, 128), I32)))
        safe = jnp.logical_and(jnp.min(lmin) >= L_LO, jnp.max(amax) <= ACC_HI_BITS)

        @pl.when(jnp.logical_not(safe))
        def _():
            MT[...] = jnp.zeros((NG, 128, 128), F32)
            ZR[...] = jnp.zeros((NG, 8, 128), F32)
            lax.fori_loop(0, NSEG * NG, attn_exact, 0)

    def oproj_body(i, c, prep):
        r0, h0 = rows(i)
        fill = _Filler(prep_jobs(W1, LV_SMALL, i, 4, range(2)) + prep_jobs(W3, LV_BIG, i, 4, [4]), 40) if prep else None
        o = _up(O[pl.ds(h0, TM // 2), :]).astype(F32)
        x = X[pl.ds(r0, TM), :] + _sdot(_acombos(o, LV_SMALL), Wo, LV_SMALL, fill)
        X[pl.ds(r0, TM), :] = x
        return c

    def w1_body(i, c, prep):
        r0, h0 = rows(i)
        fill = _Filler(prep_jobs(W2, LV_SMALL, i, 4, range(2)), 40) if prep else None
        y, v = _ln(X[pl.ds(r0, TM), :])
        z = y * lax.rsqrt(v / (v + EPS) + EPS)
        h = _gelu(_sdot(_acombos(z, LV_SMALL), W1, LV_SMALL, fill))
        A[pl.ds(A_H + 8 + r0, TM), :] = pltpu.bitcast(h, I32)
        return c

    def w2_body(i, c, prep):
        r0, h0 = rows(i)
        fill = _Filler(prep_jobs(W3, LV_BIG, i, 4, [5, 6]), 40) if prep else None
        cw = D // 4
        hb = pltpu.bitcast(A[pl.ds(A_H + r0, TM + 16), :], F32)
        hs = jnp.concatenate([
            hb[7:7 + TM, 0 * cw:1 * cw],
            hb[9:9 + TM, 1 * cw:2 * cw],
            hb[6:6 + TM, 2 * cw:3 * cw],
            hb[10:10 + TM, 3 * cw:4 * cw]], axis=1)
        x = X[pl.ds(r0, TM), :]
        y, _ = _ln(x)
        x1 = y + _sdot(_acombos(hs, LV_SMALL), W2, LV_SMALL, fill)
        X[pl.ds(r0, TM), :] = x + x1
        z1, _ = _ln(x1)
        O[pl.ds(h0, TM // 2), :] = _pk(z1.astype(BF))
        return c

    def w3_body(i, c, prep):
        r0, h0 = rows(i)
        fill = _Filler(prep_jobs(W4, LV_BIG, i, 14, range(2)), 40) if prep else None
        z1 = _up(O[pl.ds(h0, TM // 2), :]).astype(F32)
        t = _pk(_gelu(_sdot(_acombos(z1, LV_BIG), W3, LV_BIG, fill)).astype(BF))
        fq = F // 4
        for q in range(4):
            A[pl.ds(A_T[q] + h0, TM // 2), pl.ds(0, fq)] = t[:, q * fq:(q + 1) * fq]
        return c

    def w4_body(i, c, last):
        r0, h0 = rows(i)
        fq = F // 4
        t = jnp.concatenate([_up(A[pl.ds(A_T[q] + h0, TM // 2), pl.ds(0, fq)]) for q in range(4)], axis=1).astype(F32)
        xn = X[pl.ds(r0, TM), :] + _sdot(_acombos(t, LV_BIG), W4, LV_BIG)
        if last:
            O[pl.ds(h0, TM // 2), :] = _pk(xn.astype(BF))
            pltpu.make_async_copy(O.at[pl.ds(h0, TM // 2)], out32.at[pl.ds(h0, TM // 2)], osem.at[i]).start()
        else:
            X[pl.ds(r0, TM), :] = xn
        return c

    for layer in range(2):
        with jax.named_scope("qkv"):
            lax.fori_loop(0, NB, qkv_body, 0)
        if layer == 0:
            for i in range(3, 8):
                wait(i)
        with jax.named_scope("attn"):
            attn_phase(layer == 0)
        with jax.named_scope("oproj"):
            lax.fori_loop(0, NB, lambda i, c: oproj_body(i, c, layer == 0), 0)
        A[pl.ds(A_H, 8), :] = jnp.zeros((8, D), I32)
        A[pl.ds(A_H + S + 8, 8), :] = jnp.zeros((8, D), I32)
        with jax.named_scope("w1"):
            lax.fori_loop(0, NB, lambda i, c: w1_body(i, c, layer == 0), 0)
        with jax.named_scope("w2"):
            lax.fori_loop(0, NB, lambda i, c: w2_body(i, c, layer == 0), 0)
        with jax.named_scope("w3"):
            lax.fori_loop(0, NB, lambda i, c: w3_body(i, c, layer == 0), 0)
        with jax.named_scope("w4"):
            lax.fori_loop(0, NB, lambda i, c: w4_body(i, c, layer == 1), 0)
    for i in range(NB):
        pltpu.make_async_copy(O.at[pl.ds(i * TM // 2, TM // 2)], out32.at[pl.ds(i * TM // 2, TM // 2)], osem.at[i]).wait()


def _wshape(k, n, level):
    return pltpu.VMEM((7 ** level * (k >> (level + 1)), n >> level), I32)


@jax.jit
def pallas_interleave_layers__memory_aug_infini_attn__mixer_s_mlp__prompt_kernel(A_x, A_wq, A_wk, A_wv, A_wo, A_beta, B_x, B_w1, B_w2, B_w3, B_w4):
    anyspec = pl.BlockSpec(memory_space=pl.ANY)
    out = pl.pallas_call(
        _kernel,
        out_shape=jax.ShapeDtypeStruct((S, D), BF),
        in_specs=[anyspec] * 5 + [pl.BlockSpec(memory_space=pltpu.VMEM)] + [anyspec] * 4,
        out_specs=anyspec,
        scratch_shapes=[
            pltpu.VMEM((S, D), F32),
            *[_wshape(D, D, LV_SMALL)] * 6,
            _wshape(D, F, LV_BIG), _wshape(F, D, LV_BIG),
            pltpu.VMEM((ARENA, D), I32),
            pltpu.VMEM((S // 2, D), I32),
            pltpu.VMEM((NG, 128, 128), F32),
            pltpu.VMEM((NG, 8, 128), F32),
            pltpu.VMEM((D, 128), F32),
            pltpu.SemaphoreType.DMA((NSEG,)),
            pltpu.SemaphoreType.DMA((8,)),
            pltpu.SemaphoreType.DMA((NB,)),
        ],
        compiler_params=pltpu.CompilerParams(vmem_limit_bytes=128 * 1024 * 1024),
    )(A_x.reshape(S, D), A_wq, A_wk, A_wv, A_wo, A_beta.reshape(1, H), B_w1, B_w2, B_w3, B_w4)
    return out.reshape(1, S, D)
```

```python
import math
import jax
import jax.numpy as jnp
from jax import lax
import jax.experimental.pallas as pl
import jax.experimental.pallas.tpu as pltpu

S, D, F, H, DH, NSEG, L = 2048, 1024, 3584, 32, 32, 4, 512
EPS = 1e-5
NG = D // 128
NT = (((1,), (1,)), ((), ()))
BF = jnp.bfloat16
F32 = jnp.float32
I32 = jnp.int32
QSCALE = (DH ** -0.5) * math.log2(math.e)
TM = 512
NB = S // TM
L_LO = 2.0 ** -60
ACC_HI_BITS = (127 + 100) << 23
LV_SMALL = 2
LV_BIG = 2
ORDER = (2, 4, 3, 1, 0, 5, 6)

A_Q, A_PQ, A_K, A_PK, A_VT = (i * (S // 2) for i in range(5))
A_H = 0
A_T = (0, 1024, 2048, 3072)
ARENA = 5 * (S // 2)


def _ln(x):
    m = jnp.mean(x, axis=-1, keepdims=True)
    xc = x - m
    v = jnp.mean(xc * xc, axis=-1, keepdims=True)
    return xc * lax.rsqrt(v + EPS), v


def _gelu(x):
    c = math.sqrt(2.0 / math.pi)
    inner = c * (x + 0.044715 * (x * x * x))
    return 0.5 * x * (1.0 + jnp.tanh(inner))


def _phi(t):
    return jnp.where(t > 0, t + 1.0, jnp.exp(t))


def _dot(a, b):
    return jnp.dot(a, b, preferred_element_type=F32)


def _dot_nt(a, b):
    return lax.dot_general(a, b, NT, preferred_element_type=F32)


def _pk(x):
    return pltpu.bitcast(x, I32)


def _up(x):
    return pltpu.bitcast(x, BF)


def _quad(a):
    m2, k2 = a.shape[0] // 2, a.shape[1] // 2
    return a[:m2, :k2], a[:m2, k2:], a[m2:, :k2], a[m2:, k2:]


def _left(a11, a12, a21, a22):
    return (a11 + a22, a21 + a22, a11, a22, a11 + a12, a21 - a11, a12 - a22)


def _right(b11, b12, b21, b22):
    return (b11 + b22, b11, b12 - b22, b21 - b11, b22, b11 + b12, b21 + b22)


def _acombos(a, level):
    if level == 0:
        return a.astype(BF)
    return [_acombos(x, level - 1) for x in _left(*_quad(a))]


class _Filler:
    def __init__(self, jobs=(), slots=1):
        self.jobs, self.slots, self.calls, self.done = list(jobs), slots, 0, 0

    def __call__(self):
        self.calls += 1
        while self.done < len(self.jobs) and self.done * self.slots < self.calls * len(self.jobs):
            self.jobs[self.done]()
            self.done += 1


def _sdot(ac, Wp, level, fill=None, base=0, top=None):
    top = level if top is None else top
    if level == 0:
        out = _dot(ac, _up(Wp[_w(Wp, top, _slot_of_product(top)[base])]))
        if fill is not None:
            fill()
        return out
    m = [None] * 7
    for i in ORDER:
        m[i] = _sdot(ac[i], Wp, level - 1, fill, base * 7 + i, top)
    m1, m2, m3, m4, m5, m6, m7 = m
    c11 = m1 + m4 - m5 + m7
    c12 = m3 + m5
    c21 = m2 + m4
    c22 = m1 - m2 + m3 + m6
    return jnp.concatenate([jnp.concatenate([c11, c12], 1), jnp.concatenate([c21, c22], 1)], 0)


def _raw_slots(level):
    n = 2 ** level
    return [(n * c + r, r, c) for c in range(n) for r in range(n)]


def _slot_of_product(level):
    n = 2 ** level
    asis = [(0, 0)]
    for _ in range(level):
        asis = [(7 * p + i, 2 * d + (i == 4)) for (p, d) in asis for i in (1, 4)]
    table = {p: n * d + d for (p, d) in asis}
    free = [s for s in range(7 ** level) if s not in table.values()]
    for p in range(7 ** level):
        if p not in table:
            table[p] = free.pop(0)
    return table


def _w(Wp, level, slot, rows=None, cols=None):
    kb = Wp.shape[0] // 7 ** level
    r = pl.ds(slot * kb, kb) if rows is None else pl.ds(slot * kb + rows[0], rows[1])
    return (r, slice(None) if cols is None else cols)


def _prep(Wp, level, rows):
    for c0 in range(0, Wp.shape[1], 256):
        _prep_strip(Wp, level, rows, pl.ds(c0, 256))


def _prep_strip(Wp, level, rows, cols):
    raw = {(r, c): (s, _up(Wp[_w(Wp, level, s, rows, cols)])) for (s, r, c) in _raw_slots(level)}
    outs = []

    def rec(blk, lv, base):
        if lv == 0:
            slot, val = blk[(0, 0)]
            if slot is None:
                outs.append((_slot_of_product(level)[base], _pk(val.astype(BF))))
            else:
                assert slot == _slot_of_product(level)[base]
            return
        hh = 2 ** (lv - 1)
        cells = [(r, c) for r in range(hh) for c in range(hh)]
        quads = [{rc: blk[(rc[0] + a * hh, rc[1] + b * hh)] for rc in cells} for a in (0, 1) for b in (0, 1)]
        for i in range(7):
            if i == 1:
                sub = quads[0]
            elif i == 4:
                sub = quads[3]
            else:
                sub = {rc: (None, _right(*[q[rc][1].astype(F32) for q in quads])[i]) for rc in cells}
            rec(sub, lv - 1, base * 7 + i)
            if lv == 1:
                pass
        if lv == 1 and level > 1:
            flush()

    def flush():
        for base, val in outs:
            Wp[_w(Wp, level, base, rows, cols)] = val
        outs.clear()
    rec(raw, level, 0)
    flush()


def _prep_loop(Wp, level, step=8):
    def body(i, c):
        _prep(Wp, level, (pl.multiple_of(i * step, step), step))
        return c
    lax.fori_loop(0, Wp.shape[0] // 7 ** level // step, body, 0)


def _kernel(x_hbm, wq_hbm, wk_hbm, wv_hbm, wo_hbm, beta_ref, w1_hbm, w2_hbm, w3_hbm, w4_hbm,
            out_hbm,
            X, Wq, Wk, Wv, Wo, W1, W2, W3, W4, A, O, MT, ZR, G, xsem, wsem, osem):
    x32 = x_hbm.bitcast(I32)
    out32 = out_hbm.bitcast(I32)
    xcp = [pltpu.make_async_copy(x32.at[pl.ds(s * L // 2, L // 2)], O.at[pl.ds(s * L // 2, L // 2)], xsem.at[s])
           for s in range(NSEG)]

    def wcps(src, dst, level, i):
        n = 2 ** level
        kb, nb = dst.shape[0] // 7 ** level, dst.shape[1]
        src = src.bitcast(I32)
        return [pltpu.make_async_copy(src.at[:, pl.ds(c * nb, nb)], dst.at[pl.ds(n * c * kb, n * kb)], wsem.at[i])
                for c in range(n)]
    weights = [(wq_hbm, Wq, LV_SMALL), (wk_hbm, Wk, LV_SMALL), (wv_hbm, Wv, LV_SMALL), (wo_hbm, Wo, LV_SMALL),
               (w1_hbm, W1, LV_SMALL), (w2_hbm, W2, LV_SMALL), (w3_hbm, W3, LV_BIG), (w4_hbm, W4, LV_BIG)]
    wcp = [wcps(src, dst, lv, i) for i, (src, dst, lv) in enumerate(weights)]

    def start(i):
        for c in wcp[i]:
            c.start()

    def wait(i):
        for c in wcp[i]:
            c.wait()
    start(0)
    xcp[0].start()
    start(1)

    b = jax.nn.sigmoid(beta_ref[...].astype(F32))
    rhead = lax.broadcasted_iota(jnp.int32, (D, H), 0) // DH
    chead = lax.broadcasted_iota(jnp.int32, (D, H), 1)
    gcol = jnp.sum(jnp.where(rhead == chead, b, 0.0), axis=1, keepdims=True)
    G[...] = jnp.broadcast_to(gcol, (D, 128))

    wait(0)
    start(2)
    _prep_loop(Wq, LV_SMALL)
    xcp[0].wait()
    X[pl.ds(0, L), :] = _up(O[pl.ds(0, L // 2), :]).astype(F32)
    wait(1)
    for s in range(1, NSEG):
        xcp[s].start()
    _prep_loop(Wk, LV_SMALL)
    wait(2)
    _prep_loop(Wv, LV_SMALL)

    def prep_jobs(Wp, lv, i, n, strips):
        return [(lambda u=u, c=c: _prep_strip(Wp, lv, (pl.multiple_of((i * n + u) * 8, 8), 8), pl.ds(128 * c[0], 128 * c[1])))
                for u in range(n) for c in strips]

    def rows(i):
        return pl.multiple_of(i * TM, TM), pl.multiple_of(i * (TM // 2), TM // 2)

    def qkv_body(i, c, first):
        r0, h0 = rows(i)
        xn, _ = _ln(X[pl.ds(r0, TM), :])
        ac = _acombos(xn, LV_SMALL)
        q = _sdot(ac, Wq, LV_SMALL)
        A[pl.ds(A_Q + h0, TM // 2), :] = _pk((q * QSCALE).astype(BF))
        A[pl.ds(A_PQ + h0, TM // 2), :] = _pk(_phi(q).astype(BF))
        k = _sdot(ac, Wk, LV_SMALL)
        A[pl.ds(A_K + h0, TM // 2), :] = _pk(k.astype(BF))
        A[pl.ds(A_PK + h0, TM // 2), :] = _pk(_phi(k).astype(BF))
        v = _sdot(ac, Wv, LV_SMALL)
        vr = pl.multiple_of(A_VT + (i // 2) * (D // 2), D // 2)
        vc = pl.multiple_of((i % 2) * TM, TM)
        A[pl.ds(vr, D // 2), pl.ds(vc, TM)] = _pk(v.T.astype(BF))
        if first:
            @pl.when(i == 0)
            def _():
                for s in range(1, NSEG):
                    xcp[s].wait()
                    X[pl.ds(s * L, L), :] = _up(O[pl.ds(s * L // 2, L // 2), :]).astype(F32)
                for w in range(3, 8):
                    start(w)
        return c

    def consts():
        lane_head = lax.broadcasted_iota(jnp.int32, (64, 128), 1) // DH
        row_i = lax.broadcasted_iota(jnp.int32, (128, 128), 0)
        col_i = lax.broadcasted_iota(jnp.int32, (128, 128), 1)
        causal = jnp.concatenate([row_i <= col_i] * 4, axis=1)
        diag_blk = (row_i // DH) == (col_i // DH)
        zmask = lax.broadcasted_iota(jnp.int32, (8, 128), 0) == lax.broadcasted_iota(jnp.int32, (8, 128), 1) // DH
        return lane_head, causal, diag_blk, zmask

    def vt(e0, n_e, r0, n_k):
        if isinstance(r0, int):
            return _up(A[pl.ds(A_VT + (r0 // D) * (D // 2) + e0, n_e), pl.ds(r0 % D, n_k)])
        vr = pl.multiple_of(A_VT + (r0 // D) * (D // 2) + e0, 16)
        return _up(A[pl.ds(vr, n_e), pl.ds(pl.multiple_of(r0 % D, 128), n_k)])

    def scores(cs, h0, c0, j):
        lane_head, causal, _, _ = cs
        qj = A[pl.ds(A_Q + h0 + 64 * j, 64), pl.ds(c0, 128)]
        qm = _up(jnp.concatenate([jnp.where(lane_head == h, qj, 0) for h in range(4)], axis=0))
        kk = _up(A[pl.ds(A_K + h0, 64 * (j + 1)), pl.ds(c0, 128)])
        st = _dot_nt(kk, qm)
        tiles = [st[128 * t:128 * (t + 1)] for t in range(j + 1)]
        tiles[j] = jnp.where(causal, tiles[j], -1e30)
        return tiles

    def pv(tiles, m, e0, r0):
        ones = jnp.ones((16, 128), BF)
        acc = [None] * 4
        for t, tile in enumerate(tiles):
            for h in range(4):
                x = tile[:, 128 * h:128 * (h + 1)]
                if m is not None:
                    x = x - m[:, 128 * h:128 * (h + 1)]
                p = jnp.exp2(x).astype(BF)
                lv = jnp.concatenate([vt(e0 + 16 * h, 16, r0 + 128 * t, 128), ones], axis=0)
                ol = _dot(lv, p)[:DH + 8]
                acc[h] = ol if t == 0 else acc[h] + ol
        return acc

    def mem_read(mt, zr, h0, c0):
        lhs = jnp.concatenate([mt, zr, jnp.zeros((8, 128), F32)], axis=0).astype(BF)
        nd = _dot_nt(lhs, _up(A[pl.ds(A_PQ + h0, L // 2), pl.ds(c0, 128)]))
        rden = 1.0 / (nd[128:136] + 1e-6)
        rden_b = jnp.concatenate([jnp.broadcast_to(rden[h:h + 1], (DH, L)) for h in range(4)], axis=0)
        return nd[:128] * rden_b

    def mem_update(cs, mt, zr, h0, c0, e0, r0):
        _, _, diag_blk, zmask = cs
        vg = vt(e0, 64, r0, L)
        upd = _dot(jnp.concatenate([vg, jnp.ones((16, L), BF)], axis=0),
                   _up(A[pl.ds(A_PK + h0, L // 2), pl.ds(c0, 128)]))
        dm = jnp.where(diag_blk, upd[:128], 0.0)
        dz = jnp.where(zmask, upd[128:136], 0.0)
        return (dm, dz) if mt is None else (mt + dm, zr + dz)

    def store_o(ot, h0, c0, j):
        O[pl.ds(h0 + 64 * j, 64), pl.ds(c0, 128)] = _pk(ot.T.astype(BF))

    def attn_fast(g, carry, prep):
        lmin, amax = carry
        cs = consts()
        c0 = pl.multiple_of(g * 128, 128)
        e0 = pl.multiple_of(g * 64, 64)
        gt = G[pl.ds(c0, 128), :]
        mt = zr = None
        fill = _Filler()
        if prep:
            fill = _Filler(prep_jobs(Wo, LV_SMALL, g, 2, [(0, 2)]) + prep_jobs(W3, LV_BIG, g, 2, [(0, 2), (2, 2)]) + prep_jobs(W4, LV_BIG, g, 7, [(0, 1)]), 16)
        for s in range(NSEG):
            r0, h0 = s * L, s * (L // 2)
            cols = {}
            for j in (3, 2, 1, 0):
                tl = scores(cs, h0, c0, j)
                if j == 0 and s > 0:
                    amem = mem_read(mt, zr, h0, c0)
                acc = pv(tl, None, e0, r0)
                fill()
                for a in acc:
                    lmin = jnp.minimum(lmin, a[DH:])
                    ab = pltpu.bitcast(a, I32) & 0x7FFFFFFF
                    for r in range(5):
                        amax = jnp.maximum(amax, ab[8 * r:8 * r + 8])
                cols[j] = jnp.concatenate([a[:DH] * (1.0 / a[DH:DH + 1]) for a in acc], axis=0)
            for j in range(4):
                if s > 0:
                    ot = gt * amem[:, 128 * j:128 * (j + 1)] + (1.0 - gt) * cols[j]
                else:
                    ot = (1.0 - gt) * cols[j]
                store_o(ot, h0, c0, j)
            if s < NSEG - 1:
                mt, zr = mem_update(cs, mt, zr, h0, c0, e0, r0)
        return lmin, amax

    def attn_exact(idx, c):
        s = idx // NG
        g = idx % NG
        cs = consts()
        r0 = pl.multiple_of(s * L, L)
        h0 = pl.multiple_of(s * (L // 2), L // 2)
        c0 = pl.multiple_of(g * 128, 128)
        e0 = pl.multiple_of(g * 64, 64)
        gt = G[pl.ds(c0, 128), :]
        amem = mem_read(MT[g], ZR[g], h0, c0)
        for j in range(4):
            tl = scores(cs, h0, c0, j)
            mx = tl[0]
            for t in tl[1:]:
                mx = jnp.maximum(mx, t)
            m = jnp.max(mx, axis=0, keepdims=True)
            acc = pv(tl, m, e0, r0)
            col = jnp.concatenate([a[:DH] * (1.0 / a[DH:DH + 1]) for a in acc], axis=0)
            store_o(gt * amem[:, 128 * j:128 * (j + 1)] + (1.0 - gt) * col, h0, c0, j)
        MT[g], ZR[g] = mem_update(cs, MT[g], ZR[g], h0, c0, e0, r0)
        return c

    def attn_phase(prep):
        lmin, amax = lax.fori_loop(0, NG, lambda g, carry: attn_fast(g, carry, prep),
                                   (jnp.full((8, 128), 1.0, F32), jnp.zeros((8, 128), I32)))
        safe = jnp.logical_and(jnp.min(lmin) >= L_LO, jnp.max(amax) <= ACC_HI_BITS)

        @pl.when(jnp.logical_not(safe))
        def _():
            MT[...] = jnp.zeros((NG, 128, 128), F32)
            ZR[...] = jnp.zeros((NG, 8, 128), F32)
            lax.fori_loop(0, NSEG * NG, attn_exact, 0)

    def oproj_body(i, c, prep):
        r0, h0 = rows(i)
        fill = _Filler(prep_jobs(W1, LV_SMALL, i, 4, [(0, 2)]) + prep_jobs(W3, LV_BIG, i, 4, [(4, 1)]), 40) if prep else None
        o = _up(O[pl.ds(h0, TM // 2), :]).astype(F32)
        x = X[pl.ds(r0, TM), :] + _sdot(_acombos(o, LV_SMALL), Wo, LV_SMALL, fill)
        X[pl.ds(r0, TM), :] = x
        return c

    def w1_body(i, c, prep):
        r0, h0 = rows(i)
        fill = _Filler(prep_jobs(W2, LV_SMALL, i, 4, [(0, 2)]), 40) if prep else None
        y, v = _ln(X[pl.ds(r0, TM), :])
        z = y * lax.rsqrt(v / (v + EPS) + EPS)
        h = _gelu(_sdot(_acombos(z, LV_SMALL), W1, LV_SMALL, fill))
        A[pl.ds(A_H + 8 + r0, TM), :] = pltpu.bitcast(h, I32)
        return c

    def w2_body(i, c, prep):
        r0, h0 = rows(i)
        fill = _Filler(prep_jobs(W3, LV_BIG, i, 4, [(5, 2)]), 40) if prep else None
        cw = D // 4
        hb = pltpu.bitcast(A[pl.ds(A_H + r0, TM + 16), :], F32)
        hs = jnp.concatenate([
            hb[7:7 + TM, 0 * cw:1 * cw],
            hb[9:9 + TM, 1 * cw:2 * cw],
            hb[6:6 + TM, 2 * cw:3 * cw],
            hb[10:10 + TM, 3 * cw:4 * cw]], axis=1)
        x = X[pl.ds(r0, TM), :]
        y, _ = _ln(x)
        x1 = y + _sdot(_acombos(hs, LV_SMALL), W2, LV_SMALL, fill)
        X[pl.ds(r0, TM), :] = x + x1
        z1, _ = _ln(x1)
        O[pl.ds(h0, TM // 2), :] = _pk(z1.astype(BF))
        return c

    def w3_body(i, c, prep):
        r0, h0 = rows(i)
        fill = _Filler(prep_jobs(W4, LV_BIG, i, 14, [(1, 1)]), 40) if prep else None
        z1 = _up(O[pl.ds(h0, TM // 2), :]).astype(F32)
        t = _pk(_gelu(_sdot(_acombos(z1, LV_BIG), W3, LV_BIG, fill)).astype(BF))
        fq = F // 4
        for q in range(4):
            A[pl.ds(A_T[q] + h0, TM // 2), pl.ds(0, fq)] = t[:, q * fq:(q + 1) * fq]
        return c

    def w4_body(i, c, last):
        r0, h0 = rows(i)
        fq = F // 4
        t = jnp.concatenate([_up(A[pl.ds(A_T[q] + h0, TM // 2), pl.ds(0, fq)]) for q in range(4)], axis=1).astype(F32)
        xn = X[pl.ds(r0, TM), :] + _sdot(_acombos(t, LV_BIG), W4, LV_BIG)
        if last:
            O[pl.ds(h0, TM // 2), :] = _pk(xn.astype(BF))
            pltpu.make_async_copy(O.at[pl.ds(h0, TM // 2)], out32.at[pl.ds(h0, TM // 2)], osem.at[i]).start()
        else:
            X[pl.ds(r0, TM), :] = xn
        return c

    for layer in range(2):
        with jax.named_scope("qkv"):
            lax.fori_loop(0, NB, lambda i, c: qkv_body(i, c, layer == 0), 0)
        if layer == 0:
            for i in range(3, 8):
                wait(i)
        with jax.named_scope("attn"):
            attn_phase(layer == 0)
        with jax.named_scope("oproj"):
            lax.fori_loop(0, NB, lambda i, c: oproj_body(i, c, layer == 0), 0)
        A[pl.ds(A_H, 8), :] = jnp.zeros((8, D), I32)
        A[pl.ds(A_H + S + 8, 8), :] = jnp.zeros((8, D), I32)
        with jax.named_scope("w1"):
            lax.fori_loop(0, NB, lambda i, c: w1_body(i, c, layer == 0), 0)
        with jax.named_scope("w2"):
            lax.fori_loop(0, NB, lambda i, c: w2_body(i, c, layer == 0), 0)
        with jax.named_scope("w3"):
            lax.fori_loop(0, NB, lambda i, c: w3_body(i, c, layer == 0), 0)
        with jax.named_scope("w4"):
            lax.fori_loop(0, NB, lambda i, c: w4_body(i, c, layer == 1), 0)
    for i in range(NB):
        pltpu.make_async_copy(O.at[pl.ds(i * TM // 2, TM // 2)], out32.at[pl.ds(i * TM // 2, TM // 2)], osem.at[i]).wait()


def _wshape(k, n, level):
    return pltpu.VMEM((7 ** level * (k >> (level + 1)), n >> level), I32)


@jax.jit
def pallas_interleave_layers__memory_aug_infini_attn__mixer_s_mlp__prompt_kernel(A_x, A_wq, A_wk, A_wv, A_wo, A_beta, B_x, B_w1, B_w2, B_w3, B_w4):
    anyspec = pl.BlockSpec(memory_space=pl.ANY)
    out = pl.pallas_call(
        _kernel,
        out_shape=jax.ShapeDtypeStruct((S, D), BF),
        in_specs=[anyspec] * 5 + [pl.BlockSpec(memory_space=pltpu.VMEM)] + [anyspec] * 4,
        out_specs=anyspec,
        scratch_shapes=[
            pltpu.VMEM((S, D), F32),
            *[_wshape(D, D, LV_SMALL)] * 6,
            _wshape(D, F, LV_BIG), _wshape(F, D, LV_BIG),
            pltpu.VMEM((ARENA, D), I32),
            pltpu.VMEM((S // 2, D), I32),
            pltpu.VMEM((NG, 128, 128), F32),
            pltpu.VMEM((NG, 8, 128), F32),
            pltpu.VMEM((D, 128), F32),
            pltpu.SemaphoreType.DMA((NSEG,)),
            pltpu.SemaphoreType.DMA((8,)),
            pltpu.SemaphoreType.DMA((NB,)),
        ],
        compiler_params=pltpu.CompilerParams(vmem_limit_bytes=128 * 1024 * 1024),
    )(A_x.reshape(S, D), A_wq, A_wk, A_wv, A_wo, A_beta.reshape(1, H), B_w1, B_w2, B_w3, B_w4)
    return out.reshape(1, S, D)
```
